```python
import os as _os
_os.environ.setdefault("JAX_PLATFORMS", "cpu")
import jax
import jax.numpy as jnp

def _softmax(x, axis=-1):
    return jax.nn.softmax(x, axis=axis)
def _gelu(x):
    return jax.nn.gelu(x, approximate=True)
def _silu(x):
    return jax.nn.silu(x)
def _sigmoid(x):
    return jax.nn.sigmoid(x)
def _layernorm(x, axis=-1, eps=1e-5):
    m = jnp.mean(x, axis=axis, keepdims=True)
    v = jnp.var(x, axis=axis, keepdims=True)
    return (x - m) / jnp.sqrt(v + eps)
def _scatter_add(tgt, idx, src, axis=0):
    return tgt.at[idx].add(src)
def _segment_sum(src, seg, n):
    return jax.ops.segment_sum(src, seg, n)
class _Rng:
    def __init__(self, key):
        self._k = key
    def _next(self):
        self._k, sub = jax.random.split(self._k)
        return sub
    def normal(self, shape):
        return jax.random.normal(self._next(), shape, dtype=jnp.bfloat16)
    def randint(self, lo, hi, shape):
        return jax.random.randint(self._next(), shape, lo, hi, dtype=jnp.int32)
    def uniform(self, shape, lo=0.0, hi=1.0):
        return jax.random.uniform(self._next(), shape, jnp.bfloat16, lo, hi)
    def permutation(self, n):
        return jax.random.permutation(self._next(), n)


kernel_name = 'sequential_preLN__linear_kernel_hedgehog__glu_gated_swiglu__prompt'

def setup_inputs():
    _rng = _Rng(jax.random.key(int.from_bytes(__import__("os").urandom(4), "little")))
    _w = (lambda a: (lambda t: t.astype(jnp.bfloat16) if jnp.issubdtype(t.dtype, jnp.floating) else t)(jnp.asarray(a)))
    def _A_setup():
        B, S, D, H = 1, 2048, 640, 32
        Dh = D // H
        return {
            "x": _w((lambda *s: _rng.normal(s) * 0.05)(B, S, D)),
            "wqkv": _w((lambda *s: _rng.normal(s) * 0.2)(D, 3 * D)),
            "w_phi": _w((lambda *s: _rng.normal(s) * 0.2)(H, Dh, Dh) * (Dh ** -0.5)),
            "wo": _w((lambda *s: _rng.normal(s) * 0.05)(D, D)),
        }
    _A_in = _A_setup()

    def _B_setup():
        B, S, D, F = 1, 2048, 640, 1536
        return {
            "x": _w((lambda *s: _rng.normal(s) * 0.05)(B, S, D)),
            "w1": _w((lambda *s: _rng.normal(s) * 0.05)(D, F) * (2.0 / D) ** 0.5),
            "w3": _w((lambda *s: _rng.normal(s) * 0.05)(D, F) * (2.0 / D) ** 0.5),
            "w2": _w((lambda *s: _rng.normal(s) * 0.05)(F, D) * (2.0 / F) ** 0.5),
        }
    _B_in = _B_setup()

    return {
        "A_x": _A_in["x"],
        "A_wqkv": _A_in["wqkv"],
        "A_w_phi": _A_in["w_phi"],
        "A_wo": _A_in["wo"],
        "B_x": _B_in["x"],
        "B_w1": _B_in["w1"],
        "B_w3": _B_in["w3"],
        "B_w2": _B_in["w2"],
    }

def reference(A_x, A_wqkv, A_w_phi, A_wo, B_x, B_w1, B_w3, B_w2):
    def _A_ref(x, wqkv, w_phi, wo):
        B, S, D = x.shape
        H = 32; Dh = D // H
        qkv = (lambda x, *d: x.transpose(*d))((x @ wqkv).reshape(B, S, 3, H, Dh), 2, 0, 3, 1, 4)
        q, k, v = qkv[0], qkv[1], qkv[2]
        pq = jnp.einsum("bhsd,hdf->bhsf", q, w_phi)
        pk = jnp.einsum("bhsd,hdf->bhsf", k, w_phi)
        phi_q = jnp.concatenate([_softmax(pq, axis=-1), _softmax(-pq, axis=-1)], axis=-1)
        phi_k = jnp.concatenate([_softmax(pk, axis=-1), _softmax(-pk, axis=-1)], axis=-1)
        kv = jnp.einsum("bhsf,bhsd->bhfd", phi_k, v)
        z  = jnp.einsum("bhsf->bhf", phi_k)
        num = jnp.einsum("bhqf,bhfd->bhqd", phi_q, kv)
        den = jnp.einsum("bhqf,bhf->bhq", phi_q, z)[..., None] + 1e-6
        o = num / den
        return (lambda x, *d: x.transpose(*d))(o, 0, 2, 1, 3).reshape(B, S, D) @ wo

    def _B_ref(x, w1, w3, w2):
        gate = jnp.einsum("bsd,df->bsf", x, w1)
        up = jnp.einsum("bsd,df->bsf", x, w3)
        h = _silu(gate) * up
        out = jnp.einsum("bsf,fd->bsd", h, w2)
        return out

    x = A_x
    h = x + _A_ref(_layernorm(x, axis=-1), A_wqkv, A_w_phi, A_wo)
    h2 = h + _B_ref(_layernorm(h, axis=-1), B_w1, B_w3, B_w2)
    return h2
```

```python
import functools
import jax
import jax.numpy as jnp
from jax import lax
import jax.experimental.pallas as pl
import jax.experimental.pallas.tpu as pltpu

S, D, H, DH, F = 2048, 640, 32, 20, 1536
NG = 16
BF = jnp.bfloat16
F32 = jnp.float32
U32 = jnp.uint32

NT = (((1,), (1,)), ((), ()))
NN = (((1,), (0,)), ((), ()))
TN = (((0,), (0,)), ((), ()))

VB = tuple(320 * u + b for u in range(2) for b in (0, 32, 112, 160, 240))
VL = (80, 128, 96, 128, 80) * 2
FB = (0, 112, 240, 352, 480)
FL = (160, 176, 160, 176, 160)


def _dot(a, b, dims):
    return lax.dot_general(a, b, dims, preferred_element_type=F32)


def _ln(x):
    m = jnp.mean(x, axis=-1, keepdims=True)
    xc = x - m
    v = jnp.mean(xc * xc, axis=-1, keepdims=True)
    return xc * lax.rsqrt(v + 1e-5)


def _red(x, op, red):
    r = red(x, axis=1)
    r = op(r, pltpu.roll(r, 2, 1))
    r = op(r, pltpu.roll(r, 4, 1))
    return r[:, None]


def _exps(p, T):
    p4 = p.reshape(NG, 5, 8, T)
    mx = _red(p4, jnp.maximum, jnp.max)
    mn = _red(p4, jnp.minimum, jnp.min)
    ep = jnp.exp(p4 - mx)
    en = jnp.exp(mn - p4)
    sp = _red(ep, jnp.add, jnp.sum)
    sn = _red(en, jnp.add, jnp.sum)
    return ep, en, sp, sn


def _overlap_add(parts, bases, lens, total):
    cuts = sorted(set([0, total] + list(bases) + [b + l for b, l in zip(bases, lens)]))
    out = []
    for lo, hi in zip(cuts[:-1], cuts[1:]):
        acc = None
        for p, b, l in zip(parts, bases, lens):
            if b <= lo and hi <= b + l:
                piece = p[lo - b:hi - b]
                acc = piece if acc is None else acc + piece
        out.append(acc)
    return jnp.concatenate(out, axis=0)


def _pk(x):
    return pltpu.bitcast(x.astype(BF), U32)


def _upk(x):
    return pltpu.bitcast(x, BF)


def make(T1=256, T2=256):
    n1 = S // T1
    n2 = S // T2

    def kernel(x_hbm, wqkv_hbm, wphi_ref, wo_hbm, w1_hbm, w3_hbm, w2_hbm, out_hbm,
               x_v, xn_v, wqkv_v, wo_v, w1_v, w3_v, w2_v, wt_v, a2_v, kv_acc, z_acc, kvm_v, zb_v,
               h_v, hn_v, out_v, sem_x, sem_w, sem_o):
        def xcp(i):
            return pltpu.make_async_copy(x_hbm.at[pl.ds(i * T1, T1)], x_v.at[pl.ds(i * T1, T1)], sem_x.at[i])

        def wcp(j):
            return pltpu.make_async_copy(wqkv_hbm.at[:, pl.ds(j * D, D)], wqkv_v.at[j], sem_w.at[j])

        c_wo = pltpu.make_async_copy(wo_hbm, wo_v, sem_w.at[3])
        c_w1 = pltpu.make_async_copy(w1_hbm, w1_v, sem_w.at[4])
        c_w3 = pltpu.make_async_copy(w3_hbm, w3_v, sem_w.at[5])
        c_w2 = pltpu.make_async_copy(w2_hbm, w2_v, sem_w.at[6])
        xcp(0).start()
        wcp(1).start()
        wcp(2).start()
        for i in range(1, n1):
            xcp(i).start()
        wcp(0).start()

        a2_v[...] = jnp.zeros(a2_v.shape, F32)
        a2_v[:, 0:DH, :] = wphi_ref[...].astype(F32)
        a2 = a2_v[...].reshape(DH * 24, H).astype(BF)
        col = lax.broadcasted_iota(jnp.int32, (H, D), 1)
        hrow = lax.broadcasted_iota(jnp.int32, (H, D), 0)
        xsel = jnp.where((col >= hrow * DH) & (col < hrow * DH + DH), 1.0, 0.0).astype(BF)
        r = _dot(a2, xsel, NN).reshape(DH, 24, D)
        col = lax.broadcasted_iota(jnp.int32, (24, D), 1)
        dcol = col - DH * ((col * 3277) >> 16)
        u = r[0]
        for d in range(1, DH):
            u = jnp.where(dcol == d, r[d], u)
        ub = jnp.concatenate([u, jnp.zeros((8, D), F32)], axis=0).astype(BF)
        dup = (lax.broadcasted_iota(jnp.int32, (48, 32), 0) >> 1) == lax.broadcasted_iota(jnp.int32, (48, 32), 1)
        u2 = _dot(jnp.where(dup, 1.0, 0.0).astype(BF), ub, NN)[0:2 * DH].reshape(1, 5, 8, D)
        sh = (NG, 1, 8, D)
        hh = lax.broadcasted_iota(jnp.int32, sh, 0) * 2 + (lax.broadcasted_iota(jnp.int32, sh, 2) & 1)
        cc = lax.broadcasted_iota(jnp.int32, sh, 3)
        msk = (cc >= hh * DH) & (cc < hh * DH + DH)
        bdt = jnp.where(msk, u2, 0.0).reshape(D, D).astype(BF)

        def fold(j):
            parts = [_dot(bdt[FB[t]:FB[t] + FL[t], 128 * t:128 * (t + 1)],
                          wqkv_v[j, :, 128 * t:128 * (t + 1)], NT) for t in range(5)]
            wt_v[j] = _pk(_overlap_add(parts, FB, FL, D))

        def ln1(i, r0):
            xcp(i).wait()
            x = x_v[pl.ds(r0, T1), :].astype(F32)
            return _pk(_ln(x))

        xn_v[0:T1 // 2, :] = ln1(0, 0)
        wcp(1).wait()
        fold(1)
        wcp(2).wait()
        eye = (lax.broadcasted_iota(jnp.int32, (128, 128), 0) == lax.broadcasted_iota(jnp.int32, (128, 128), 1))
        eye = jnp.where(eye, 1.0, 0.0).astype(BF)
        for t in range(D // 128):
            wt_v[2, t * 64:(t + 1) * 64, :] = _pk(_dot(eye, wqkv_v[2, :, t * 128:(t + 1) * 128], NT))
        c_wo.start()
        c_w1.start()
        c_w3.start()
        c_w2.start()
        kv_acc[...] = jnp.zeros(kv_acc.shape, F32)
        z_acc[...] = jnp.zeros(z_acc.shape, F32)

        def b1(xn):
            pk = _dot(_upk(wt_v[1]), xn, NT)
            vt = _dot(_upk(wt_v[2]), xn, NT).astype(BF)
            ep, en, sp, sn = _exps(pk, T1)
            phi = jnp.concatenate([ep * (1.0 / sp), en * (1.0 / sn)], axis=1).reshape(2 * D, T1)
            zs = phi[:, 0:128]
            for c in range(1, T1 // 128):
                zs = zs + phi[:, c * 128:(c + 1) * 128]
            z_acc[...] += zs
            phib = phi.astype(BF)
            for t in range(10):
                kv_acc[t, 0:VL[t], :] += _dot(vt[VB[t]:VB[t] + VL[t]], phib[128 * t:128 * (t + 1)], NT)

        def p1(i, carry):
            win = xn_v.at[pl.ds(pl.multiple_of(i * (T1 // 2), T1 // 2), T1)]
            xn = _upk(win[0:T1 // 2, :])
            win[T1 // 2:T1, :] = ln1(i + 1, pl.multiple_of((i + 1) * T1, T1))
            b1(xn)
            return carry

        lax.fori_loop(0, n1 - 1, p1, 0)
        b1(_upk(xn_v[(n1 - 1) * T1 // 2:n1 * T1 // 2, :]))

        wcp(0).wait()
        fold(0)
        for t in range(10):
            rr = lax.broadcasted_iota(jnp.int32, (VL[t], 128), 0) + VB[t]
            p = lax.broadcasted_iota(jnp.int32, (VL[t], 128), 1) + 128 * t
            hp = 2 * ((p * 52429) >> 22) + (p & 1)
            mg = (rr >= hp * DH) & (rr < hp * DH + DH)
            kvm_v[t, 0:VL[t] // 2, :] = _pk(jnp.where(mg, kv_acc[t, 0:VL[t], :], 0.0))
        zb_v[...] = jnp.broadcast_to(jnp.sum(z_acc[...], axis=1, keepdims=True), zb_v.shape)
        c_wo.wait()

        def ocp(i, slot):
            return pltpu.make_async_copy(out_v.at[slot], out_hbm.at[pl.ds(i * T2, T2)], sem_o.at[slot])

        def a2(xn, x):
            pq = _dot(_upk(wt_v[0]), xn, NT)
            ep, en, sp, sn = _exps(pq, T2)
            zb = zb_v[...].reshape(NG, 10, 8, 128)
            zb = jnp.concatenate([zb] * (T2 // 128), axis=3)
            rp = 1.0 / sp
            rn = 1.0 / sn
            dd = jnp.sum(ep * zb[:, :5], axis=1, keepdims=True) * rp + jnp.sum(en * zb[:, 5:], axis=1, keepdims=True) * rn
            rden = 1.0 / (_red(dd, jnp.add, jnp.sum) + 1e-6)
            phib = jnp.concatenate([ep * (rp * rden), en * (rn * rden)], axis=1).reshape(2 * D, T2).astype(BF)
            parts = [_dot(_upk(kvm_v[t, 0:VL[t] // 2, :]), phib[128 * t:128 * (t + 1)], NN) for t in range(10)]
            ot = _overlap_add(parts, VB, VL, D)
            attn = _dot(ot.astype(BF), wo_v[...], TN)
            h = x.astype(F32) + attn
            return h, _pk(_ln(h))

        def b2(h, hn):
            gate = _dot(hn, w1_v[...], NN)
            up = _dot(hn, w3_v[...], NN)
            act = (gate * (0.5 * jnp.tanh(0.5 * gate) + 0.5) * up).astype(BF)
            return (h + _dot(act, w2_v[...], NN)).astype(BF)

        h0, hn0 = a2(_upk(xn_v[0:T2 // 2, :]), x_v[0:T2, :])
        h_v[0:T2, :] = h0
        hn_v[0:T2 // 2, :] = hn0
        c_w1.wait()
        c_w3.wait()
        c_w2.wait()

        def p2(i, carry):
            slot = i % 2
            r1 = pl.multiple_of((i + 1) * T2, T2)
            hw = h_v.at[pl.ds(pl.multiple_of(i * T2, T2), 2 * T2)]
            hnw = hn_v.at[pl.ds(pl.multiple_of(i * (T2 // 2), T2 // 2), T2)]

            @pl.when(i >= 2)
            def _():
                ocp(i - 2, slot).wait()

            h1, hn1 = a2(_upk(xn_v[pl.ds(pl.multiple_of((i + 1) * (T2 // 2), T2 // 2), T2 // 2), :]),
                         x_v[pl.ds(r1, T2), :])
            hw[T2:2 * T2, :] = h1
            hnw[T2 // 2:T2, :] = hn1
            y = b2(hw[0:T2, :], _upk(hnw[0:T2 // 2, :]))
            out_v[slot] = y
            ocp(i, slot).start()
            return carry

        lax.fori_loop(0, n2 - 1, p2, 0)
        last = n2 - 1
        ocp(last - 2, last % 2).wait()
        out_v[last % 2] = b2(h_v[last * T2:(last + 1) * T2, :], _upk(hn_v[last * T2 // 2:(last + 1) * T2 // 2, :]))
        ocp(last, last % 2).start()
        ocp(last - 1, (last - 1) % 2).wait()
        ocp(last, last % 2).wait()

    def fn(A_x, A_wqkv, A_w_phi, A_wo, B_x, B_w1, B_w3, B_w2):
        any_spec = pl.BlockSpec(memory_space=pl.ANY)
        out = pl.pallas_call(
            kernel,
            out_shape=jax.ShapeDtypeStruct((S, D), BF),
            in_specs=[any_spec, any_spec, pl.BlockSpec(memory_space=pltpu.VMEM), any_spec, any_spec, any_spec, any_spec],
            out_specs=any_spec,
            scratch_shapes=[
                pltpu.VMEM((S, D), BF),
                pltpu.VMEM((S // 2, D), U32),
                pltpu.VMEM((3, D, D), BF),
                pltpu.VMEM((D, D), BF),
                pltpu.VMEM((D, F), BF),
                pltpu.VMEM((D, F), BF),
                pltpu.VMEM((F, D), BF),
                pltpu.VMEM((3, D // 2, D), U32),
                pltpu.VMEM((DH, 24, H), F32),
                pltpu.VMEM((10, 128, 128), F32),
                pltpu.VMEM((2 * D, 128), F32),
                pltpu.VMEM((10, 64, 128), U32),
                pltpu.VMEM((2 * D, 128), F32),
                pltpu.VMEM((S, D), F32),
                pltpu.VMEM((S // 2, D), U32),
                pltpu.VMEM((2, T2, D), BF),
                pltpu.SemaphoreType.DMA((n1,)),
                pltpu.SemaphoreType.DMA((7,)),
                pltpu.SemaphoreType.DMA((2,)),
            ],
            compiler_params=pltpu.CompilerParams(vmem_limit_bytes=100 * 1024 * 1024),
        )(A_x.reshape(S, D), A_wqkv, A_w_phi.transpose(1, 2, 0), A_wo, B_w1, B_w3, B_w2)
        return out.reshape(1, S, D)
    return fn


_impl = make()


@jax.jit
def pallas_sequential_preLN__linear_kernel_hedgehog__glu_gated_swiglu__prompt_kernel(
    A_x: jax.Array,
    A_wqkv: jax.Array,
    A_w_phi: jax.Array,
    A_wo: jax.Array,
    B_x: jax.Array,
    B_w1: jax.Array,
    B_w3: jax.Array,
    B_w2: jax.Array,
):
    return _impl(A_x, A_wqkv, A_w_phi, A_wo, B_x, B_w1, B_w3, B_w2)
```

```python
import functools
import jax
import jax.numpy as jnp
from jax import lax
import jax.experimental.pallas as pl
import jax.experimental.pallas.tpu as pltpu

S, D, H, DH, F = 2048, 640, 32, 20, 1536
NG = 16
BF = jnp.bfloat16
F32 = jnp.float32
LOG2E = 1.4426950408889634

NT = (((1,), (1,)), ((), ()))
NN = (((1,), (0,)), ((), ()))
TN = (((0,), (0,)), ((), ()))

VB = tuple(320 * u + b for u in range(2) for b in (0, 32, 112, 160, 240))
VL = (80, 128, 96, 128, 80) * 2
FB = (0, 112, 240, 352, 480)
FL = (160, 176, 160, 176, 160)


def _dot(a, b, dims):
    return lax.dot_general(a, b, dims, preferred_element_type=F32)


def _ln(x):
    m = jnp.mean(x, axis=-1, keepdims=True)
    xc = x - m
    v = jnp.mean(xc * xc, axis=-1, keepdims=True)
    return xc * lax.rsqrt(v + 1e-5)


def _red(x, op, red):
    r = red(x, axis=1)
    r = op(r, pltpu.roll(r, 2, 1))
    r = op(r, pltpu.roll(r, 4, 1))
    return r[:, None]


def _rcp(x):
    r = pl.reciprocal(x, approx=True)
    return r * (2.0 - x * r)


def _exps(p):
    p4 = p.reshape(p.shape[0] // 40, 5, 8, p.shape[1])
    mx = _red(p4, jnp.maximum, jnp.max)
    mn = _red(p4, jnp.minimum, jnp.min)
    ep = jnp.exp2(p4 - mx)
    en = jnp.exp2(mn - p4)
    sp = _red(ep, jnp.add, jnp.sum)
    sn = _red(en, jnp.add, jnp.sum)
    return ep, en, sp, sn


def _overlap_add(parts, bases, lens, total):
    cuts = sorted(set([0, total] + list(bases) + [b + l for b, l in zip(bases, lens)]))
    out = []
    for lo, hi in zip(cuts[:-1], cuts[1:]):
        acc = None
        for p, b, l in zip(parts, bases, lens):
            if b <= lo and hi <= b + l:
                piece = p[lo - b:hi - b]
                acc = piece if acc is None else acc + piece
        out.append(acc)
    return jnp.concatenate(out, axis=0)


class _Scope:
    def __init__(self, on):
        self.on = on
        self.cur = None

    def __call__(self, name):
        if not self.on:
            return
        if self.cur is not None:
            self.cur.__exit__(None, None, None)
        self.cur = None
        if name is not None:
            self.cur = jax.named_scope(name)
            self.cur.__enter__()


def make(T=256, FC=512, DS=256, SC=0, LASTSPLIT=2, KS=384, MC=160, EAGER=1, WOFF=0, BQ=6):
    n = S // T

    def kernel(x_hbm, wqkv_hbm, wphi_hbm, wo_hbm, w1_hbm, w3_hbm, w2_hbm, out_hbm,
               x_v, wqkv_v, wphi_v, wo_v, w1_v, w3_v, w2_v, a2_v,
               out_v, sem_x, sem_w, sem_k, sem_o, sem_f):
        sc = _Scope(SC)

        def xcp(i):
            return pltpu.make_async_copy(x_hbm.at[pl.ds(i * T, T)], x_v.at[pl.ds(i * T, T)], sem_x.at[i])

        def wcp(j):
            return pltpu.make_async_copy(wqkv_hbm.at[:, pl.ds(j * D, D)], wqkv_v.at[j], sem_w.at[j])

        def kcp(t):
            c0, c1 = (0, KS) if t == 0 else (KS, D)
            return pltpu.make_async_copy(wqkv_hbm.at[:, pl.ds(D + c0, c1 - c0)],
                                         wqkv_v.at[1, :, pl.ds(c0, c1 - c0)], sem_k.at[t])

        c_ph = pltpu.make_async_copy(wphi_hbm, wphi_v, sem_w.at[1])
        c_wo = pltpu.make_async_copy(wo_hbm, wo_v, sem_w.at[3])
        c_w1 = pltpu.make_async_copy(w1_hbm, w1_v, sem_w.at[4])
        c_w3 = pltpu.make_async_copy(w3_hbm, w3_v, sem_w.at[5])
        c_w2 = pltpu.make_async_copy(w2_hbm, w2_v, sem_w.at[6])
        sc('prologue')
        order = [c_ph, kcp(0), xcp(0), kcp(1), wcp(2)] + [xcp(i) for i in range(1, n)] + [wcp(0), c_wo, c_w1, c_w3, c_w2]
        for c in order:
            c.start()
            pl.semaphore_signal(sem_f, 1)
            pl.semaphore_wait(sem_f, 1)

        a2_v[...] = jnp.zeros(a2_v.shape, F32)
        c_ph.wait()
        sc('bdt')
        a2_v[:, 0:DH, :] = wphi_v[...].astype(F32)
        a2 = a2_v[...].reshape(DH * 24, H).astype(BF)
        col = lax.broadcasted_iota(jnp.int32, (H, D), 1)
        hrow = lax.broadcasted_iota(jnp.int32, (H, D), 0)
        xsel = jnp.where((col >= hrow * DH) & (col < hrow * DH + DH), 1.0, 0.0).astype(BF)
        r = _dot(a2, xsel, NN).reshape(DH, 24, D)
        col = lax.broadcasted_iota(jnp.int32, (24, D), 1)
        dcol = col - DH * ((col * 3277) >> 16)
        u = r[0]
        for d in range(1, DH):
            u = jnp.where(dcol == d, r[d], u)
        ub = jnp.concatenate([u, jnp.zeros((8, D), F32)], axis=0).astype(BF)
        dup = (lax.broadcasted_iota(jnp.int32, (48, 32), 0) >> 1) == lax.broadcasted_iota(jnp.int32, (48, 32), 1)
        u2 = _dot(jnp.where(dup, 1.0, 0.0).astype(BF), ub, NN)[0:2 * DH].reshape(1, 5, 8, D)
        sh = (NG, 1, 8, D)
        hh = lax.broadcasted_iota(jnp.int32, sh, 0) * 2 + (lax.broadcasted_iota(jnp.int32, sh, 2) & 1)
        cc = lax.broadcasted_iota(jnp.int32, sh, 3)
        msk = (cc >= hh * DH) & (cc < hh * DH + DH)
        bdf = jnp.where(msk, u2, 0.0).reshape(D, D)
        bdt = [bdf[FB[t]:FB[t] + FL[t], 128 * t:128 * (t + 1)].astype(BF) for t in range(5)]

        def fold_part(j, t):
            return _dot(bdt[t], wqkv_v[j, :, 128 * t:128 * (t + 1)], NT)

        def ln1(i):
            return _ln(x_v[i * T:(i + 1) * T, :].astype(F32)).astype(BF)

        NP = D // MC

        def msplit(w):
            return [w[c * MC:(c + 1) * MC].astype(BF) for c in range(NP)]

        class Soft:
            def __init__(self, fn):
                self.fn, self.ps, self.tiles, self.pend, self.rows, self.g = fn, [], [], [], 0, 0

            def add(self, p):
                self.ps.append(p)
                if EAGER and self.fn() is not None:
                    while self.g < len(self.ps) * (MC // 40):
                        self.step()

            def step(self):
                c, a = divmod(self.g * 40, MC)
                self.pend.append(self.fn()(self.g, self.ps[c][a:a + 40]))
                self.g += 1
                self.rows += 80
                if self.rows >= 128:
                    cat = jnp.concatenate(self.pend, axis=0)
                    self.tiles.append(cat[0:128].astype(BF))
                    self.rows -= 128
                    self.pend = [cat[128:]] if self.rows else []

            def tile(self, t):
                while len(self.tiles) <= t:
                    self.step()
                return self.tiles[t]

        zacc = [None] * NG
        zb = [None] * NG
        zcnt = [0] * NG

        def fk(g, p):
            ep, en, sp, sn = _exps(p)
            r = _rcp(sp * sn)
            phi = jnp.concatenate([ep * (r * sn), en * (r * sp)], axis=1).reshape(80, T)
            zs = phi[:, 0:128]
            for c in range(1, T // 128):
                zs = zs + phi[:, c * 128:(c + 1) * 128]
            zacc[g] = zs if zacc[g] is None else zacc[g] + zs
            zcnt[g] += 1
            if zcnt[g] == n:
                zb[g] = jnp.broadcast_to(jnp.sum(zacc[g], axis=1, keepdims=True), (80, 128)).reshape(1, 10, 8, 128)
            return phi

        def fq(g, p):
            ep, en, sp, sn = _exps(p)
            z = jnp.concatenate([zb[g]] * (T // 128), axis=3)
            dd = jnp.sum(ep * z[:, :5], axis=1, keepdims=True) * sn + jnp.sum(en * z[:, 5:], axis=1, keepdims=True) * sp
            r = _rcp(_red(dd, jnp.add, jnp.sum) + 1e-6 * (sp * sn))
            return jnp.concatenate([ep * (r * sn), en * (r * sp)], axis=1).reshape(80, T)

        sk = [Soft(lambda: fk) for _ in range(n)]
        sq = [Soft(lambda: fq if zb[NG - 1] is not None else None) for _ in range(n)]
        vts = [[] for _ in range(n)]
        vws = [[] for _ in range(n)]
        kvacc = [None] * 10
        kvm = [None] * 10
        W = {}
        xn = {}

        def kp(i, c):
            sk[i].add(_dot(W['k'][c], xn[i], NT))

        def qp(i, c):
            sq[i].add(_dot(W['q'][c], xn[i], NT))

        def vp(i, c):
            vts[i].append(_dot(W['v'][c], xn[i], NT))
            while len(vws[i]) < 10 and VB[len(vws[i])] + VL[len(vws[i])] <= (c + 1) * MC:
                t = len(vws[i])
                vt = jnp.concatenate(vts[i], axis=0)
                vws[i].append(vt[VB[t]:VB[t] + VL[t]].astype(BF))

        def kv(i, t):
            new = _dot(vws[i][t], sk[i].tile(t), NT)
            kvacc[t] = new if kvacc[t] is None else kvacc[t] + new
            if i == n - 1:
                rr = lax.broadcasted_iota(jnp.int32, (VL[t], 128), 0) + VB[t]
                p = lax.broadcasted_iota(jnp.int32, (VL[t], 128), 1) + 128 * t
                hp = 2 * ((p * 52429) >> 22) + (p & 1)
                mg = (rr >= hp * DH) & (rr < hp * DH + DH)
                kvm[t] = jnp.where(mg, kvacc[t], 0.0).astype(BF)

        nparts = [[] for _ in range(n)]

        def nm(i, t):
            nparts[i].append(_dot(kvm[t], sq[i].tile(t), NN))

        def P(f, i, cnt):
            return [functools.partial(f, i, c) for c in range(cnt)]

        def weave(big, small):
            k = 0
            for j, f in enumerate(big):
                f()
                while k < len(small) and (k + 1) * len(big) <= (j + 1) * len(small) + WOFF:
                    small[k]()
                    k += 1
            while k < len(small):
                small[k]()
                k += 1

        sc('w_ka')
        kcp(0).wait()
        sc('folda')
        parts = [fold_part(1, t) for t in range(KS // 128)]
        sc('w_kb')
        xcp(0).wait()
        kcp(1).wait()
        sc('foldb')
        xn[0] = ln1(0)
        parts += [fold_part(1, t) for t in range(KS // 128, 5)]
        W['k'] = msplit(_overlap_add(parts, FB, FL, D) * LOG2E)
        weave(P(kp, 0, NP), [])
        sc('w_v')
        wcp(2).wait()
        xcp(1).wait()
        sc('p1a')
        eye = (lax.broadcasted_iota(jnp.int32, (128, 128), 0) == lax.broadcasted_iota(jnp.int32, (128, 128), 1))
        eye = jnp.where(eye, 1.0, 0.0).astype(BF)
        W['v'] = msplit(jnp.concatenate([_dot(eye, wqkv_v[2, :, t * 128:(t + 1) * 128], NT) for t in range(5)], axis=0))
        xn[1] = ln1(1)
        weave(P(vp, 0, NP), [])
        for i in range(1, n):
            if i == BQ:
                sc('p1c')
                wcp(0).wait()
                c_wo.wait()
                c_w1.wait()
                c_w3.wait()
                c_w2.wait()
                W['q'] = msplit(_overlap_add([fold_part(0, t) for t in range(5)], FB, FL, D) * LOG2E)
            kvs = P(kv, i - 1, 10)
            weave(P(kp, i, NP), kvs[:5])
            if i == 1:
                sc('p1b')
                for k in range(2, n):
                    xcp(k).wait()
            if i + 1 < n:
                xn[i + 1] = ln1(i + 1)
            weave(P(vp, i, NP), kvs[5:])
        weave(P(qp, 0, NP) + P(qp, 1, NP), P(kv, n - 1, 10))
        weave(P(qp, 2, NP) + P(qp, 3, NP), P(nm, 0, 10))

        def num(i):
            return _overlap_add(nparts[i], VB, VL, D).astype(BF)

        def wo(ot, i):
            h = x_v[i * T:(i + 1) * T, :].astype(F32) + _dot(ot, wo_v[...], TN)
            return h, _ln(h).astype(BF)

        def gu(hn, rs=1):
            acts = [[] for _ in range(rs)]
            R = T // rs
            for c in range(F // FC):
                gate = _dot(hn, w1_v[:, c * FC:(c + 1) * FC], NN)
                up = _dot(hn, w3_v[:, c * FC:(c + 1) * FC], NN)
                hg = 0.5 * gate
                a = hg * (jnp.tanh(hg) + 1.0) * up
                for k in range(rs):
                    acts[k].append(a[k * R:(k + 1) * R].astype(BF))
            return acts

        def dn(h, act, i, c0, c1, r0=0, r1=T):
            y = h[r0:r1, c0:c1]
            for c in range(F // FC):
                y = y + _dot(act[c], w2_v[c * FC:(c + 1) * FC, c0:c1], NN)
            out_v[i * T + r0:i * T + r1, c0:c1] = y.astype(BF)

        ocps = []

        def ocp(r0, r1):
            c = pltpu.make_async_copy(out_v.at[pl.ds(r0, r1 - r0)], out_hbm.at[pl.ds(r0, r1 - r0)], sem_o.at[len(ocps)])
            ocps.append(c)
            c.start()

        sc('mid')
        weave(P(qp, 4, NP), [])
        h, hn = wo(num(0), 0)
        weave(P(qp, 5, NP), P(nm, 1, 10))
        sc('p2')
        for i in range(n):
            if i + 1 < n:
                act = gu(hn)[0]
                dn(h, act, i, 0, DS)
                h1, hn1 = wo(num(i + 1), i + 1)
                if i + 2 < n:
                    weave(P(nm, i + 2, 10), [])
                dn(h, act, i, DS, D)
                ocp(i * T, (i + 1) * T)
                if i + 6 < n:
                    weave(P(qp, i + 6, NP), [])
                h, hn = h1, hn1
            else:
                acts = gu(hn, LASTSPLIT)
                RS = T // LASTSPLIT
                for k in range(LASTSPLIT):
                    dn(h, acts[k], i, 0, D, k * RS, (k + 1) * RS)
                    ocp(i * T + k * RS, i * T + (k + 1) * RS)
        sc('fin')
        for c in ocps:
            c.wait()
        sc(None)

    def fn(A_x, A_wqkv, A_w_phi, A_wo, B_x, B_w1, B_w3, B_w2):
        any_spec = pl.BlockSpec(memory_space=pl.ANY)
        out = pl.pallas_call(
            kernel,
            out_shape=jax.ShapeDtypeStruct((S, D), BF),
            in_specs=[any_spec] * 7,
            out_specs=any_spec,
            scratch_shapes=[
                pltpu.VMEM((S, D), BF),
                pltpu.VMEM((3, D, D), BF),
                pltpu.VMEM((DH, DH, H), BF),
                pltpu.VMEM((D, D), BF),
                pltpu.VMEM((D, F), BF),
                pltpu.VMEM((D, F), BF),
                pltpu.VMEM((F, D), BF),
                pltpu.VMEM((DH, 24, H), F32),
                pltpu.VMEM((S, D), BF),
                pltpu.SemaphoreType.DMA((n,)),
                pltpu.SemaphoreType.DMA((7,)),
                pltpu.SemaphoreType.DMA((2,)),
                pltpu.SemaphoreType.DMA((n - 1 + LASTSPLIT,)),
                pltpu.SemaphoreType.REGULAR,
            ],
            compiler_params=pltpu.CompilerParams(vmem_limit_bytes=100 * 1024 * 1024),
        )(A_x.reshape(S, D), A_wqkv, A_w_phi.transpose(1, 2, 0), A_wo, B_w1, B_w3, B_w2)
        return out.reshape(1, S, D)
    return fn


_impl = make()


@jax.jit
def pallas_sequential_preLN__linear_kernel_hedgehog__glu_gated_swiglu__prompt_kernel(
    A_x: jax.Array,
    A_wqkv: jax.Array,
    A_w_phi: jax.Array,
    A_wo: jax.Array,
    B_x: jax.Array,
    B_w1: jax.Array,
    B_w3: jax.Array,
    B_w2: jax.Array,
):
    return _impl(A_x, A_wqkv, A_w_phi, A_wo, B_x, B_w1, B_w3, B_w2)
```

```python
import functools
import jax
import jax.numpy as jnp
from jax import lax
import jax.experimental.pallas as pl
import jax.experimental.pallas.tpu as pltpu

S, D, H, DH, F = 2048, 640, 32, 20, 1536
NG = 16
BF = jnp.bfloat16
F32 = jnp.float32
LOG2E = 1.4426950408889634

NT = (((1,), (1,)), ((), ()))
NN = (((1,), (0,)), ((), ()))
TN = (((0,), (0,)), ((), ()))

FB = (0, 112, 240, 352, 480)
FL = (160, 176, 160, 176, 160)


def _dot(a, b, dims):
    return lax.dot_general(a, b, dims, preferred_element_type=F32)


def _ln(x, x2=None):
    m = jnp.mean(x, axis=-1, keepdims=True)
    xc = x - m
    v = jnp.mean(xc * xc, axis=-1, keepdims=True)
    r = lax.rsqrt(v + 1e-5)
    if x2 is None:
        return xc * r
    return x2() * r - m * r


def _red(x, op, red):
    r = red(x, axis=1)
    r = op(r, pltpu.roll(r, 2, 1))
    r = op(r, pltpu.roll(r, 4, 1))
    return r[:, None]


def _rcp(x):
    r = pl.reciprocal(x, approx=True)
    return r * (2.0 - x * r)


def _phi(p):
    p4 = p.reshape(1, 5, 8, p.shape[1])
    mx = _red(p4, jnp.maximum, jnp.max)
    mn = _red(p4, jnp.minimum, jnp.min)
    ep = jnp.exp2(p4 - mx)
    en = jnp.exp2(mn - p4)
    sp = _red(ep, jnp.add, jnp.sum)
    sn = _red(en, jnp.add, jnp.sum)
    r = _rcp(sp * sn)
    return jnp.concatenate([ep * (r * sn), en * (r * sp)], axis=1).reshape(80, p.shape[1]).astype(BF)


def _overlap_add(parts, bases, lens, total):
    cuts = sorted(set([0, total] + list(bases) + [b + l for b, l in zip(bases, lens)]))
    out = []
    for lo, hi in zip(cuts[:-1], cuts[1:]):
        acc = None
        for p, b, l in zip(parts, bases, lens):
            if b <= lo and hi <= b + l:
                piece = p[lo - b:hi - b]
                acc = piece if acc is None else acc + piece
        out.append(acc)
    return jnp.concatenate(out, axis=0)


class _Scope:
    def __init__(self, on):
        self.on = on
        self.cur = None

    def __call__(self, name):
        if not self.on:
            return
        if self.cur is not None:
            self.cur.__exit__(None, None, None)
        self.cur = None
        if name is not None:
            self.cur = jax.named_scope(name)
            self.cur.__enter__()


DMAS = "x0:1 k0:384|k384:640 x1:2|x2:4 v0:640|x4:8 q0:640"
SCHED = ("w1 fk0:3 l0 k0.0:2h w2 fk3:5 l1 k0.2:4 k1h w3 tv l2 v0 k2 l3 v1 k3 v2 w4 fq l4 v3 k4 l5 v4 k5 l6 v5 k6 l7 v6 k7 v7 "
         "q0 q1 q2 q3 q4 q5 q6 q7")


def make(T=256, FC=512, SC=0, MC=160, LOOP=1, XV=0, GS=3, U=1, XT=1, DEF=1, LAGK=2, LAGV=1, LAGQ=4, RK=4, RN=5, CHK=0,
         EV=2, LNM=0, LG=2, RB=16, DMAS=DMAS, SCHED=SCHED):
    n = S // T
    R = T // 2

    def kernel(x_hbm, wqkv_hbm, wphi_hbm, wo_hbm, w1_hbm, w3_hbm, w2_hbm, out_hbm,
               x_v, wqkv_v, wphi_v, wo_v, w1_v, w3_v, w2_v, a2_v, o_v,
               out_v, sem_i, sem_o, sem_f):
        sc = _Scope(SC)

        def xcp(i0, i1, s):
            return pltpu.make_async_copy(x_hbm.at[pl.ds(i0 * T, (i1 - i0) * T)], x_v.at[pl.ds(i0 * T, (i1 - i0) * T)], sem_i.at[s])

        def wcp(j, c0, c1, s):
            return pltpu.make_async_copy(wqkv_hbm.at[:, pl.ds(j * D + c0, c1 - c0)],
                                         wqkv_v.at[j, :, pl.ds(c0, c1 - c0)], sem_i.at[s])

        def mkcp(tok, s):
            lo, hi = map(int, tok[1:].split(':'))
            return xcp(lo, hi, s) if tok[0] == 'x' else wcp('qkv'.index(tok[0]), lo, hi, s)

        groups = [[pltpu.make_async_copy(wphi_hbm, wphi_v, sem_i.at[0])]]
        for grp in DMAS.split('|'):
            groups.append([mkcp(tok, len(groups)) for tok in grp.split()])
        groups.append([pltpu.make_async_copy(a, b, sem_i.at[len(groups)])
                       for a, b in ((wo_hbm, wo_v), (w1_hbm, w1_v), (w3_hbm, w3_v), (w2_hbm, w2_v))])
        sc('prologue')
        for grp in groups:
            for c in grp:
                c.start()
                pl.semaphore_signal(sem_f, 1)
                pl.semaphore_wait(sem_f, 1)

        def wait(k):
            sc('w%d' % k)
            for c in groups[k]:
                c.wait()
            sc('c%d' % k)

        a2_v[...] = jnp.zeros(a2_v.shape, F32)
        wait(0)
        a2_v[:, 0:DH, :] = wphi_v[...].astype(F32)
        a2 = a2_v[...].reshape(DH * 24, H).astype(BF)
        col = lax.broadcasted_iota(jnp.int32, (H, D), 1)
        hrow = lax.broadcasted_iota(jnp.int32, (H, D), 0)
        xsel = jnp.where((col >= hrow * DH) & (col < hrow * DH + DH), 1.0, 0.0).astype(BF)
        r = _dot(a2, xsel, NN).reshape(DH, 24, D)
        col = lax.broadcasted_iota(jnp.int32, (24, D), 1)
        dcol = col - DH * ((col * 3277) >> 16)
        u = r[0]
        for d in range(1, DH):
            u = jnp.where(dcol == d, r[d], u)
        ub = jnp.concatenate([u, jnp.zeros((8, D), F32)], axis=0).astype(BF)
        dup = (lax.broadcasted_iota(jnp.int32, (48, 32), 0) >> 1) == lax.broadcasted_iota(jnp.int32, (48, 32), 1)
        u2 = _dot(jnp.where(dup, 1.0, 0.0).astype(BF), ub, NN)[0:2 * DH].reshape(1, 5, 8, D)
        sh = (NG, 1, 8, D)
        hh = lax.broadcasted_iota(jnp.int32, sh, 0) * 2 + (lax.broadcasted_iota(jnp.int32, sh, 2) & 1)
        cc = lax.broadcasted_iota(jnp.int32, sh, 3)
        msk = (cc >= hh * DH) & (cc < hh * DH + DH)
        bdf = jnp.where(msk, u2, 0.0).reshape(D, D)
        bdt = [bdf[FB[t]:FB[t] + FL[t], 128 * t:128 * (t + 1)].astype(BF) for t in range(5)]

        def fold_part(j, t):
            return _dot(bdt[t], wqkv_v[j, :, 128 * t:128 * (t + 1)], NT)

        def ln1(i):
            if LG and i >= 2:
                outs, rs = [], []
                for k in range(T // RB):
                    x = x_v[i * T + k * RB:i * T + (k + 1) * RB, :].astype(F32)
                    c = 1.0 / D if k < LG else jnp.minimum(1.0 / D, rs[k - LG] + 1.0)
                    xc = x - jnp.sum(x, axis=-1, keepdims=True) * c
                    r = lax.rsqrt(jnp.mean(xc * xc, axis=-1, keepdims=True) + 1e-5)
                    rs.append(r)
                    outs.append(xc * r)
                return jnp.concatenate(outs, axis=0).astype(BF)
            ld = lambda: x_v[i * T:(i + 1) * T, :].astype(F32)
            return _ln(ld(), ld if LNM else None).astype(BF)

        NP = D // MC
        GP = MC // 40

        phk = [[] for _ in range(n)]
        phq = [[] for _ in range(n)]
        vws = [[] for _ in range(n)]
        kvacc = [None] * NG
        kvm = [None] * NG
        W = {}
        xn = {}
        ones8 = jnp.ones((8, T), F32)

        pend = []

        def flush():
            for dst, p in pend:
                dst += [_phi(p[40 * g:40 * (g + 1)]) for g in range(p.shape[0] // 40)]
            pend.clear()

        def proj(kind, i, c, half=False):
            w = W[kind][c]
            ws = [w[0:MC // 2], w[MC // 2:MC]] if half else [w]
            for w in ws:
                p = _dot(w.astype(BF), xn[i], NT)
                if kind == 'v':
                    vws[i] += [jnp.concatenate([p[40 * g:40 * (g + 1)], ones8], axis=0).astype(BF)
                               for g in range(p.shape[0] // 40)]
                else:
                    pend.append(((phk if kind == 'k' else phq)[i], p))

        rr = lax.broadcasted_iota(jnp.int32, (48, 80), 0)
        pp = lax.broadcasted_iota(jnp.int32, (48, 80), 1)
        hr = jnp.where(((rr >= DH) & (rr < 2 * DH)) | (rr >= 2 * DH + 4), 1, 0)
        mg = hr == (pp & 1)

        def kv(i, g):
            new = _dot(vws[i][g], phk[i][g], NT)
            kvacc[g] = new if kvacc[g] is None else kvacc[g] + new
            if i == n - 1:
                kvm[g] = jnp.where(mg, kvacc[g], 0.0).astype(BF)

        nparts = [[] for _ in range(n)]
        lo4 = lax.broadcasted_iota(jnp.int32, (8, T), 0) < 4

        def nm(i, g):
            t = _dot(kvm[g], phq[i][g], NN)
            ra = _rcp(t[40:48] + 1e-6)
            rb = pltpu.roll(ra, 4, 0)
            r0 = jnp.where(lo4, ra, rb)
            r1 = jnp.where(lo4, rb, ra)
            nparts[i].append(t[0:40] * jnp.concatenate([r0, r0, ra, r1, r1], axis=0))
            if g == NG - 1:
                ot = jnp.concatenate(nparts[i], axis=0)
                if XT == 1:
                    o_v[i * T:(i + 1) * T, :] = ot.astype(BF).T
                else:
                    o_v[i * T:(i + 1) * T, :] = ot.T.astype(BF)

        def wsplit(parts, lo, hi):
            m = len(parts)
            w = _overlap_add(parts, FB[:m], FL[:m], FB[m - 1] + FL[m - 1])
            return [w[c * MC:(c + 1) * MC] * LOG2E for c in range(lo, hi)]

        done = {}
        st = {'j': 0, 'kv': 0, 'nm': 0}
        kvdone = {}

        def smalls(final=False):
            j = st['j']
            cnt = 0
            while st['kv'] < n * NG and (final or cnt < RK * EV):
                i, g = divmod(st['kv'], NG)
                if not final and (done.get(('k', i, g // GP), 1 << 20) + LAGK > j or done.get(('v', i, g // GP), 1 << 20) + LAGV > j):
                    break
                kv(i, g)
                if i == n - 1:
                    kvdone[g] = j
                st['kv'] += 1
                cnt += 1
            while st['nm'] < n * NG and (final or cnt < RN * EV):
                i, g = divmod(st['nm'], NG)
                if not final and (kvdone.get(g, 1 << 20) + 1 > j or done.get(('q', i, g // GP), 1 << 20) + LAGQ > j):
                    break
                nm(i, g)
                st['nm'] += 1
                cnt += 1

        parts = {'k': [], 'q': []}
        W['k'], W['q'] = [], []
        toks = SCHED.split()
        for ti, tok in enumerate(toks):
            nxt = toks[ti + 1] if ti + 1 < len(toks) else ''
            if tok[0] == 'w':
                wait(int(tok[1:]))
            elif tok[0] == 's':
                sc(tok)
            elif tok[0] == 'f':
                kind = tok[1]
                lo, hi = map(int, tok[2:].split(':')) if len(tok) > 2 else (0, 5)
                parts[kind] += [fold_part('qk'.index(kind), t) for t in range(lo, hi)]
                W[kind] += wsplit(parts[kind], len(W[kind]), FB[hi] // MC if hi < 5 else NP)
                flush()
            elif tok == 'tv':
                if XV:
                    wvt = wqkv_v[2].T
                else:
                    eye = (lax.broadcasted_iota(jnp.int32, (128, 128), 0) == lax.broadcasted_iota(jnp.int32, (128, 128), 1))
                    eye = jnp.where(eye, 1.0, 0.0).astype(BF)
                    wvt = jnp.concatenate([_dot(eye, wqkv_v[2, :, t * 128:(t + 1) * 128], NT) for t in range(5)], axis=0)
                W['v'] = [wvt[c * MC:(c + 1) * MC] for c in range(NP)]
                flush()
            elif tok[0] == 'l':
                xn[int(tok[1:])] = ln1(int(tok[1:]))
            else:
                half = tok.endswith('h')
                allh = tok.endswith('H')
                t2 = tok.rstrip('hH')
                i = int(t2[1:].split('.')[0])
                lo, hi = map(int, t2.split('.')[1].split(':')) if '.' in t2 else (0, NP)
                for c in range(lo, hi):
                    proj(tok[0], i, c, allh or (half and c == hi - 1))
                    if not (nxt.startswith('w') and c >= hi - DEF):
                        flush()
                    done[(tok[0], i, c)] = st['j']
                    if st['j'] % EV == EV - 1:
                        smalls()
                    st['j'] += 1
        smalls(True)
        wait(len(groups) - 1)

        def ocp(r0, k):
            return pltpu.make_async_copy(out_v.at[pl.ds(r0, R)], out_hbm.at[pl.ds(r0, R)], sem_o)

        def gu(hn, c):
            gate = _dot(hn, w1_v[:, c * FC:(c + 1) * FC], NN)
            up = _dot(hn, w3_v[:, c * FC:(c + 1) * FC], NN)
            hg = 0.5 * gate
            return hg * (jnp.tanh(hg) + 1.0) * up

        def chunk(i):
            rows = [i * T + k * R if isinstance(i, int) else pl.multiple_of(i * T + k * R, R) for k in range(2)]
            hs, hns = [], []
            for k in range(2):
                h = x_v[pl.ds(rows[k], R), :].astype(F32) + _dot(o_v[pl.ds(rows[k], R), :], wo_v[...], NN)
                hs.append(h)
                hns.append(_ln(h, (lambda: h) if LNM > 1 else None))
            acts = [[], []]
            hb = [hns[k].astype(BF) for k in range(2)]
            for k in range(2):
                for c in range(GS):
                    acts[k].append(gu(hb[k], c).astype(BF))
            if GS < F // FC:
                hf = jnp.concatenate(hns, axis=0).astype(BF)
                for c in range(GS, F // FC):
                    a = gu(hf, c)
                    for k in range(2):
                        acts[k].append(a[k * R:(k + 1) * R].astype(BF))
            for k in range(2):
                y = hs[k]
                for c in range(F // FC):
                    y = y + _dot(acts[k][c], w2_v[c * FC:(c + 1) * FC, :], NN)
                out_v[pl.ds(rows[k], R), :] = y.astype(BF)
                ocp(rows[k], 2 * i + k).start()

        sc('p2')
        if LOOP:
            def body(j, carry):
                for u in range(U):
                    chunk(j * U + u)
                return carry
            lax.fori_loop(0, n // U, body, 0)
        else:
            for i in range(n):
                chunk(i)
        sc('fin')
        pltpu.make_async_copy(out_v, out_hbm, sem_o).wait()
        sc(None)

    def fn(A_x, A_wqkv, A_w_phi, A_wo, B_x, B_w1, B_w3, B_w2):
        any_spec = pl.BlockSpec(memory_space=pl.ANY)
        out = pl.pallas_call(
            kernel,
            out_shape=jax.ShapeDtypeStruct((S, D), BF),
            in_specs=[any_spec] * 7,
            out_specs=any_spec,
            scratch_shapes=[
                pltpu.VMEM((S, D), BF),
                pltpu.VMEM((3, D, D), BF),
                pltpu.VMEM((DH, DH, H), BF),
                pltpu.VMEM((D, D), BF),
                pltpu.VMEM((D, F), BF),
                pltpu.VMEM((D, F), BF),
                pltpu.VMEM((F, D), BF),
                pltpu.VMEM((DH, 24, H), F32),
                pltpu.VMEM((S, D), BF),
                pltpu.VMEM((S, D), BF),
                pltpu.SemaphoreType.DMA((len(DMAS.split('|')) + 2,)),
                pltpu.SemaphoreType.DMA,
                pltpu.SemaphoreType.REGULAR,
            ],
            compiler_params=pltpu.CompilerParams(vmem_limit_bytes=100 * 1024 * 1024,
                                                 disable_bounds_checks=not CHK, disable_semaphore_checks=not CHK),
        )(A_x.reshape(S, D), A_wqkv, A_w_phi.transpose(1, 2, 0), A_wo, B_w1, B_w3, B_w2)
        return out.reshape(1, S, D)
    return fn


_impl = make()


@jax.jit
def pallas_sequential_preLN__linear_kernel_hedgehog__glu_gated_swiglu__prompt_kernel(
    A_x: jax.Array,
    A_wqkv: jax.Array,
    A_w_phi: jax.Array,
    A_wo: jax.Array,
    B_x: jax.Array,
    B_w1: jax.Array,
    B_w3: jax.Array,
    B_w2: jax.Array,
):
    return _impl(A_x, A_wqkv, A_w_phi, A_wo, B_x, B_w1, B_w3, B_w2)
```

```python
import functools
import jax
import jax.numpy as jnp
from jax import lax
import jax.experimental.pallas as pl
import jax.experimental.pallas.tpu as pltpu

S, D, H, DH, F = 2048, 640, 32, 20, 1536
NG = 16
BF = jnp.bfloat16
F32 = jnp.float32
LOG2E = 1.4426950408889634

NT = (((1,), (1,)), ((), ()))
NN = (((1,), (0,)), ((), ()))
TN = (((0,), (0,)), ((), ()))

FBS = ((0, 112, 240, 352, 480), (0, 120, 240, 360, 480))
FLS = ((160, 176, 160, 176, 160), (160, 160, 160, 160, 160))


def _dot(a, b, dims):
    return lax.dot_general(a, b, dims, preferred_element_type=F32)


def _ln(x, x2=None):
    m = jnp.mean(x, axis=-1, keepdims=True)
    xc = x - m
    v = jnp.mean(xc * xc, axis=-1, keepdims=True)
    r = lax.rsqrt(v + 1e-5)
    if x2 is None:
        return xc * r
    return x2() * r - m * r


def _red(x, op, red):
    r = red(x, axis=1)
    r = op(r, pltpu.roll(r, 2, 1))
    r = op(r, pltpu.roll(r, 4, 1))
    return r[:, None]


def _rcp(x):
    r = pl.reciprocal(x, approx=True)
    return r * (2.0 - x * r)


def _phi(p, gate=None):
    p4 = p.reshape(1, 5, 8, p.shape[1])
    mx = _red(p4, jnp.maximum, jnp.max)
    mn = _red(p4, jnp.minimum, jnp.min)
    if gate is not None:
        mx = jnp.maximum(mx, gate)
        mn = jnp.minimum(mn, -gate)
    ep = jnp.exp2(p4 - mx)
    en = jnp.exp2(mn - p4)
    sp = _red(ep, jnp.add, jnp.sum)
    sn = _red(en, jnp.add, jnp.sum)
    r = _rcp(sp * sn)
    return jnp.concatenate([ep * (r * sn), en * (r * sp)], axis=1).reshape(80, p.shape[1]).astype(BF)


def _overlap_add(parts, bases, lens, total):
    cuts = sorted(set([0, total] + list(bases) + [b + l for b, l in zip(bases, lens)]))
    out = []
    for lo, hi in zip(cuts[:-1], cuts[1:]):
        acc = None
        for p, b, l in zip(parts, bases, lens):
            if b <= lo and hi <= b + l:
                piece = p[lo - b:hi - b]
                acc = piece if acc is None else acc + piece
        out.append(acc)
    return jnp.concatenate(out, axis=0)


class _Scope:
    def __init__(self, on):
        self.on = on
        self.cur = None

    def __call__(self, name):
        if not self.on:
            return
        if self.cur is not None:
            self.cur.__exit__(None, None, None)
        self.cur = None
        if name is not None:
            self.cur = jax.named_scope(name)
            self.cur.__enter__()


DMAS = "x0:1|k0:384|k384:640 x1:2|x2:4 v0:640|x4:8 q0:640"
SCHED = ("w1 l0 bd w2 fk0:3 k0.0:2h w3 fk3:5 l1 k0.2:4 k1h w4 tv l2 v0 k2 l3 v1 k3 v2 w5 fq l4 v3 k4 l5 v4 k5 l6 v5 k6 l7 v6 k7 v7 "
         "q0 q1 q2 q3 q4 q5 q6 q7")


def make(T=256, FC=512, SC=0, MC=160, LOOP=1, XV=0, GS=3, U=1, XT=1, DEF=1, LAGK=2, LAGV=2, LAGQ=5, RK=4, RN=5, CHK=0,
         EV=2, LNM=0, LG=2, RB=16, DCOL=(512, 128), PT=0, UB=0, LI=2, GR=248, FBK=1, FBQ=1, LAGE=2, CE=0, DMAS=DMAS, SCHED=SCHED):
    n = S // T
    R = T // 2

    def kernel(x_hbm, wqkv_hbm, wphi_hbm, wo_hbm, w1_hbm, w3_hbm, w2_hbm, out_hbm,
               x_v, wqkv_v, wphi_v, wo_v, w1_v, w3_v, w2_v, a2_v, o_v,
               out_v, sem_i, sem_o, sem_f):
        sc = _Scope(SC)

        def xcp(i0, i1, s):
            return pltpu.make_async_copy(x_hbm.at[pl.ds(i0 * T, (i1 - i0) * T)], x_v.at[pl.ds(i0 * T, (i1 - i0) * T)], sem_i.at[s])

        def wcp(j, c0, c1, s):
            return pltpu.make_async_copy(wqkv_hbm.at[:, pl.ds(j * D + c0, c1 - c0)],
                                         wqkv_v.at[j, :, pl.ds(c0, c1 - c0)], sem_i.at[s])

        def mkcp(tok, s):
            lo, hi = map(int, tok[1:].split(':'))
            return xcp(lo, hi, s) if tok[0] == 'x' else wcp('qkv'.index(tok[0]), lo, hi, s)

        groups = [[pltpu.make_async_copy(wphi_hbm, wphi_v, sem_i.at[0])]]
        for grp in DMAS.split('|'):
            groups.append([mkcp(tok, len(groups)) for tok in grp.split()])
        groups.append([pltpu.make_async_copy(a, b, sem_i.at[len(groups)])
                       for a, b in ((wo_hbm, wo_v), (w1_hbm, w1_v), (w3_hbm, w3_v), (w2_hbm, w2_v))])
        sc('prologue')
        for grp in groups:
            for c in grp:
                c.start()
                pl.semaphore_signal(sem_f, 1)
                pl.semaphore_wait(sem_f, 1)

        def wait(k):
            sc('w%d' % k)
            for c in groups[k]:
                c.wait()
            sc('c%d' % k)

        a2_v[...] = jnp.zeros(a2_v.shape, F32)
        wait(0)
        a2_v[:, 0:DH, :] = wphi_v[...].astype(F32)
        a2 = a2_v[...].reshape(DH * 24, H).astype(BF)
        col = lax.broadcasted_iota(jnp.int32, (H, D), 1)
        hrow = lax.broadcasted_iota(jnp.int32, (H, D), 0)
        xsel = jnp.where((col >= hrow * DH) & (col < hrow * DH + DH), 1.0, 0.0).astype(BF)
        r = _dot(a2, xsel, NN).reshape(DH, 24, D)
        col = lax.broadcasted_iota(jnp.int32, (24, D), 1)
        dcol = col - DH * ((col * 3277) >> 16)
        u = r[0]
        for d in range(1, DH):
            u = jnp.where(dcol == d, r[d], u)
        ub = jnp.concatenate([u, jnp.zeros((8, D), F32)], axis=0).astype(BF)
        bdt = []

        def bd2():
            dup = (lax.broadcasted_iota(jnp.int32, (48, 32), 0) >> 1) == lax.broadcasted_iota(jnp.int32, (48, 32), 1)
            u2 = _dot(jnp.where(dup, 1.0, 0.0).astype(BF), ub, NN)[0:2 * DH].reshape(1, 5, 8, D)
            sh = (NG, 1, 8, D)
            hh = lax.broadcasted_iota(jnp.int32, sh, 0) * 2 + (lax.broadcasted_iota(jnp.int32, sh, 2) & 1)
            cc = lax.broadcasted_iota(jnp.int32, sh, 3)
            msk = (cc >= hh * DH) & (cc < hh * DH + DH)
            bdf = jnp.where(msk, u2, 0.0).reshape(D, D)
            for FB, FL in ((FBS[FBQ], FLS[FBQ]), (FBS[FBK], FLS[FBK])):
                bdt.append([bdf[FB[t]:FB[t] + FL[t], 128 * t:128 * (t + 1)].astype(BF) for t in range(5)])

        def fold_part(j, t):
            return _dot(bdt[j][t], wqkv_v[j, :, 128 * t:128 * (t + 1)], NT)

        lnr = [None]

        def ln1(i):
            if LG and i >= LI:
                outs, rs = [], []
                for k in range(T // RB):
                    x = x_v[i * T + k * RB:i * T + (k + 1) * RB, :].astype(F32)
                    c = 1.0 / D if k < LG else jnp.minimum(1.0 / D, rs[k - LG] + 1.0)
                    xc = x - jnp.sum(x, axis=-1, keepdims=True) * c
                    r = lax.rsqrt(jnp.mean(xc * xc, axis=-1, keepdims=True) + 1e-5)
                    rs.append(r)
                    outs.append(xc * r)
                lnr[0] = rs[-1][-8:]
                return jnp.concatenate(outs, axis=0).astype(BF)
            x = x_v[i * T:(i + 1) * T, :].astype(F32)
            xc = x - jnp.mean(x, axis=-1, keepdims=True)
            r = lax.rsqrt(jnp.mean(xc * xc, axis=-1, keepdims=True) + 1e-5)
            lnr[0] = r[GR:GR + 8]
            return (xc * r).astype(BF)

        NP = D // MC
        GP = MC // 40

        phk = [[] for _ in range(n)]
        phq = [[] for _ in range(n)]
        vws = [[] for _ in range(n)]
        kvacc = [None] * NG
        kvm = [None] * NG
        W = {}
        xn = {}
        ones8 = jnp.ones((8, T), F32)

        pend = []

        def flush():
            for dst, p, gate in pend:
                dst += [_phi(p[40 * g:40 * (g + 1)], gate) for g in range(p.shape[0] // 40)]
            pend.clear()

        def proj(kind, i, c, half=False, gated=False):
            w = W[kind][c]
            ws = [w[0:MC // 2], w[MC // 2:MC]] if half else [w]
            for w in ws:
                p = _dot(w.astype(BF), xn[i], NT)
                if kind == 'v':
                    vws[i] += [jnp.concatenate([p[40 * g:40 * (g + 1)], ones8], axis=0).astype(BF)
                               for g in range(p.shape[0] // 40)]
                else:
                    gate = jnp.minimum(lnr[0], -3e38).reshape(1, 1, 8, 1) if gated else None
                    pend.append(((phk if kind == 'k' else phq)[i], p, gate))

        rr = lax.broadcasted_iota(jnp.int32, (48, 80), 0)
        pp = lax.broadcasted_iota(jnp.int32, (48, 80), 1)
        hr = jnp.where(((rr >= DH) & (rr < 2 * DH)) | (rr >= 2 * DH + 4), 1, 0)
        mg = hr == (pp & 1)

        def kv(i, g):
            new = _dot(vws[i][g], phk[i][g], NT)
            kvacc[g] = new if kvacc[g] is None else kvacc[g] + new
            if i == n - 1:
                kvm[g] = jnp.where(mg, kvacc[g], 0.0).astype(BF)

        nparts = [[] for _ in range(n)]
        lo4 = lax.broadcasted_iota(jnp.int32, (8, T), 0) < 4

        def nm(i, g):
            t = _dot(kvm[g], phq[i][g], NN)
            ra = _rcp(t[40:48] + 1e-6)
            rb = pltpu.roll(ra, 4, 0)
            r0 = jnp.where(lo4, ra, rb)
            r1 = jnp.where(lo4, rb, ra)
            nparts[i].append(t[0:40] * jnp.concatenate([r0, r0, ra, r1, r1], axis=0))
            if PT and i >= n - PT:
                t = (40 * (g + 1)) // 128 - 1
                if (40 * g) // 128 - 1 < t:
                    ot = jnp.concatenate(nparts[i], axis=0)[128 * t:128 * (t + 1)]
                    if UB:
                        o_v[i * R:(i + 1) * R, 128 * t:128 * (t + 1)] = pltpu.bitcast(ot.astype(BF).T, jnp.uint32)
                    else:
                        o_v[i * T:(i + 1) * T, 128 * t:128 * (t + 1)] = ot.astype(BF).T
            elif g == NG - 1:
                ot = jnp.concatenate(nparts[i], axis=0).astype(BF).T
                if UB:
                    o_v[i * R:(i + 1) * R, :] = pltpu.bitcast(ot, jnp.uint32)
                else:
                    o_v[i * T:(i + 1) * T, :] = ot

        def wsplit(parts, lo, hi, FB, FL):
            m = len(parts)
            w = _overlap_add(parts, FB[:m], FL[:m], FB[m - 1] + FL[m - 1])
            return [w[c * MC:(c + 1) * MC] * LOG2E for c in range(lo, hi)]

        done = {}
        st = {'j': 0, 'kv': 0, 'nm': 0, 'e': 0}
        kvdone = {}

        def smalls(final=False):
            j = st['j']
            cnt = 0
            while st['kv'] < n * NG and (final or cnt < RK * EV):
                i, g = divmod(st['kv'], NG)
                if not final and (done.get(('k', i, g // GP), 1 << 20) + LAGK > j or done.get(('v', i, g // GP), 1 << 20) + LAGV > j):
                    break
                kv(i, g)
                if i == n - 1:
                    kvdone[g] = j
                st['kv'] += 1
                cnt += 1
            while st['nm'] < n * NG and (final or cnt < RN * EV):
                i, g = divmod(st['nm'], NG)
                if not final and (kvdone.get(g, 1 << 20) + 1 > j or done.get(('q', i, g // GP), 1 << 20) + (LAGE if st['e'] else LAGQ) > j):
                    break
                nm(i, g)
                st['nm'] += 1
                cnt += 1

        parts = {'k': [], 'q': [], 'v': []}
        W['k'], W['q'], W['v'] = [], [], []
        toks = SCHED.split()
        for ti, tok in enumerate(toks):
            nxt = toks[ti + 1] if ti + 1 < len(toks) else ''
            if tok[0] == 'w':
                wait(int(tok[1:]))
            elif tok[0] == 's':
                sc(tok)
            elif tok[0] == 'f':
                kind = tok[1]
                lo, hi = map(int, tok[2:].split(':')) if len(tok) > 2 else (0, 5)
                parts[kind] += [fold_part('qk'.index(kind), t) for t in range(lo, hi)]
                FB, FL = (FBS[FBQ], FLS[FBQ]) if kind == 'q' else (FBS[FBK], FLS[FBK])
                W[kind] += wsplit(parts[kind], len(W[kind]), FB[hi] // MC if hi < 5 else NP, FB, FL)
                flush()
            elif tok == 'bd':
                bd2()
            elif tok[:2] == 'tv':
                lo, hi = map(int, tok[2:].split(':')) if len(tok) > 2 else (0, 5)
                eye = (lax.broadcasted_iota(jnp.int32, (128, 128), 0) == lax.broadcasted_iota(jnp.int32, (128, 128), 1))
                eye = jnp.where(eye, 1.0, 0.0).astype(BF)
                parts['v'] += [_dot(eye, wqkv_v[2, :, t * 128:(t + 1) * 128], NT) for t in range(lo, hi)]
                wvt = jnp.concatenate(parts['v'], axis=0)
                W['v'] += [wvt[c * MC:(c + 1) * MC] for c in range(len(W['v']), 128 * hi // MC)]
                flush()
            elif tok[0] == 'l':
                xn[int(tok[1:])] = ln1(int(tok[1:]))
            else:
                nofl = tok.endswith('n')
                gated = tok.endswith('g')
                tok = tok.rstrip('ng')
                half = tok.endswith('h')
                allh = tok.endswith('H')
                t2 = tok.rstrip('hH')
                i = int(t2[1:].split('.')[0])
                lo, hi = map(int, t2.split('.')[1].split(':')) if '.' in t2 else (0, NP)
                for c in range(lo, hi):
                    proj(tok[0], i, c, allh or (half and c == hi - 1), gated)
                    if not (nxt.startswith('w') and c >= hi - DEF) and not nofl:
                        flush()
                    done[(tok[0], i, c)] = st['j']
                    st['e'] = tok[0] == 'q' and i * NP + c >= n * NP - CE
                    if st['j'] % EV == EV - 1 or st['e']:
                        smalls()
                    st['j'] += 1
        smalls(True)
        wait(len(groups) - 1)


        def gu(hn, c):
            gate = _dot(hn, w1_v[:, c * FC:(c + 1) * FC], NN)
            up = _dot(hn, w3_v[:, c * FC:(c + 1) * FC], NN)
            hg = 0.5 * gate
            return hg * (jnp.tanh(hg) + 1.0) * up

        def chunk(i):
            rows = [i * T + k * R if isinstance(i, int) else pl.multiple_of(i * T + k * R, R) for k in range(2)]
            orow = [pl.multiple_of(i * R + k * (R // 2), R // 2) for k in range(2)]
            hs, hns = [], []
            for k in range(2):
                h = x_v[pl.ds(rows[k], R), :].astype(F32) + _dot(pltpu.bitcast(o_v[pl.ds(orow[k], R // 2), :], BF) if UB else o_v[pl.ds(rows[k], R), :], wo_v[...], NN)
                hs.append(h)
                hns.append(_ln(h, (lambda: h) if LNM > 1 else None))
            acts = [[], []]
            hb = [hns[k].astype(BF) for k in range(2)]
            for k in range(2):
                for c in range(GS):
                    acts[k].append(gu(hb[k], c).astype(BF))
            if GS < F // FC:
                hf = jnp.concatenate(hns, axis=0).astype(BF)
                for c in range(GS, F // FC):
                    a = gu(hf, c)
                    for k in range(2):
                        acts[k].append(a[k * R:(k + 1) * R].astype(BF))
            for k in range(2):
                c0 = 0
                for cw in (DCOL if k == 1 else (D,)):
                    y = hs[k][:, c0:c0 + cw]
                    for c in range(F // FC):
                        y = y + _dot(acts[k][c], w2_v[c * FC:(c + 1) * FC, c0:c0 + cw], NN)
                    out_v[pl.ds(rows[k], R), c0:c0 + cw] = y.astype(BF)
                    pltpu.make_async_copy(out_v.at[pl.ds(rows[k], R), pl.ds(c0, cw)],
                                          out_hbm.at[pl.ds(rows[k], R), pl.ds(c0, cw)], sem_o).start()
                    c0 += cw

        sc('p2')
        if LOOP:
            def body(j, carry):
                for u in range(U):
                    chunk(j * U + u)
                return carry
            lax.fori_loop(0, n // U, body, 0)
        else:
            for i in range(n):
                chunk(i)
        sc('fin')
        pltpu.make_async_copy(out_v, out_hbm, sem_o).wait()
        sc(None)

    def fn(A_x, A_wqkv, A_w_phi, A_wo, B_x, B_w1, B_w3, B_w2):
        any_spec = pl.BlockSpec(memory_space=pl.ANY)
        out = pl.pallas_call(
            kernel,
            out_shape=jax.ShapeDtypeStruct((S, D), BF),
            in_specs=[any_spec] * 7,
            out_specs=any_spec,
            scratch_shapes=[
                pltpu.VMEM((S, D), BF),
                pltpu.VMEM((3, D, D), BF),
                pltpu.VMEM((DH, DH, H), BF),
                pltpu.VMEM((D, D), BF),
                pltpu.VMEM((D, F), BF),
                pltpu.VMEM((D, F), BF),
                pltpu.VMEM((F, D), BF),
                pltpu.VMEM((DH, 24, H), F32),
                pltpu.VMEM((S // 2, D), jnp.uint32) if UB else pltpu.VMEM((S, D), BF),
                pltpu.VMEM((S, D), BF),
                pltpu.SemaphoreType.DMA((len(DMAS.split('|')) + 2,)),
                pltpu.SemaphoreType.DMA,
                pltpu.SemaphoreType.REGULAR,
            ],
            compiler_params=pltpu.CompilerParams(vmem_limit_bytes=100 * 1024 * 1024,
                                                 disable_bounds_checks=not CHK, disable_semaphore_checks=not CHK),
        )(A_x.reshape(S, D), A_wqkv, A_w_phi.transpose(1, 2, 0), A_wo, B_w1, B_w3, B_w2)
        return out.reshape(1, S, D)
    return fn


_impl = make()


@jax.jit
def pallas_sequential_preLN__linear_kernel_hedgehog__glu_gated_swiglu__prompt_kernel(
    A_x: jax.Array,
    A_wqkv: jax.Array,
    A_w_phi: jax.Array,
    A_wo: jax.Array,
    B_x: jax.Array,
    B_w1: jax.Array,
    B_w3: jax.Array,
    B_w2: jax.Array,
):
    return _impl(A_x, A_wqkv, A_w_phi, A_wo, B_x, B_w1, B_w3, B_w2)
```

```python
import functools
import jax
import jax.numpy as jnp
from jax import lax
import jax.experimental.pallas as pl
import jax.experimental.pallas.tpu as pltpu

S, D, H, DH, F = 2048, 640, 32, 20, 1536
NG = 16
BF = jnp.bfloat16
F32 = jnp.float32
LOG2E = 1.4426950408889634

NT = (((1,), (1,)), ((), ()))
NN = (((1,), (0,)), ((), ()))
TN = (((0,), (0,)), ((), ()))

FBS = ((0, 112, 240, 352, 480), (0, 120, 240, 360, 480), (0, 120, 240, 376, 496))
FLS = ((160, 176, 160, 176, 160), (160, 160, 160, 160, 160), (144, 144, 160, 144, 144))
SPLIT = (1, 3, 6, 9, 12)
GROUPS = ((0, 1, 0), (2, 1, 1), (4, 3, 0), (5, 3, 1), (7, 6, 0), (8, 6, 1), (10, 9, 0), (11, 9, 1),
          (13, 12, 0), (14, 12, 1), (15, None, 0))
NGR = len(GROUPS)


def _dot(a, b, dims):
    return lax.dot_general(a, b, dims, preferred_element_type=F32)


def _ln(x, x2=None):
    m = jnp.mean(x, axis=-1, keepdims=True)
    xc = x - m
    v = jnp.mean(xc * xc, axis=-1, keepdims=True)
    r = lax.rsqrt(v + 1e-5)
    if x2 is None:
        return xc * r
    return x2() * r - m * r


def _red(x, op, red):
    r = red(x, axis=1)
    r = op(r, pltpu.roll(r, 2, 1))
    r = op(r, pltpu.roll(r, 4, 1))
    return r[:, None]


def _rcp(x, nw=1):
    r = pl.reciprocal(x, approx=True)
    return r * (2.0 - x * r) if nw else r


def _phi(p, gate=None, nw=1):
    p4 = p.reshape(1, 5, 8, p.shape[1])
    mx = _red(p4, jnp.maximum, jnp.max)
    mn = _red(p4, jnp.minimum, jnp.min)
    if gate is not None:
        mx = jnp.maximum(mx, gate)
        mn = jnp.minimum(mn, -gate)
    ep = jnp.exp2(p4 - mx)
    en = jnp.exp2(mn - p4)
    sp = _red(ep, jnp.add, jnp.sum)
    sn = _red(en, jnp.add, jnp.sum)
    r = _rcp(sp * sn, nw)
    return jnp.concatenate([ep * (r * sn), en * (r * sp)], axis=1).reshape(80, p.shape[1]).astype(BF)


def _phis(p, nw=1):
    ev = (lax.broadcasted_iota(jnp.int32, (8, p.shape[1]), 0) & 1) == 0

    def red(v, op):
        a, b = op(v[0], v[1]), op(v[3], v[4])
        c = op(jnp.where(ev, a, b), pltpu.roll(jnp.where(ev, b, a), 1, 0))
        c = op(c, v[2])
        c = op(c, pltpu.roll(c, 2, 0))
        return op(c, pltpu.roll(c, 4, 0))

    def spread(c):
        cr = pltpu.roll(c, 1, 0)
        a, b = jnp.where(ev, c, cr), jnp.where(ev, cr, c)
        return [a, a, c, b, b]

    v = [p[8 * j:8 * (j + 1)] for j in range(5)]
    ep = [jnp.exp2(x - m) for x, m in zip(v, spread(red(v, jnp.maximum)))]
    en = [jnp.exp2(m - x) for x, m in zip(v, spread(red(v, jnp.minimum)))]
    sp, sn = red(ep, jnp.add), red(en, jnp.add)
    r = _rcp(sp * sn, nw)
    ep = [x * m for x, m in zip(ep, spread(r * sn))]
    en = [x * m for x, m in zip(en, spread(r * sp))]
    return [jnp.concatenate(ep[0:3] + en[0:3], axis=0).astype(BF), jnp.concatenate(ep[2:5] + en[2:5], axis=0).astype(BF)]


def _overlap_add(parts, bases, lens, total):
    cuts = sorted(set([0, total] + list(bases) + [b + l for b, l in zip(bases, lens)]))
    out = []
    for lo, hi in zip(cuts[:-1], cuts[1:]):
        acc = None
        for p, b, l in zip(parts, bases, lens):
            if b <= lo and hi <= b + l:
                piece = p[lo - b:hi - b]
                acc = piece if acc is None else acc + piece
        out.append(acc)
    return jnp.concatenate(out, axis=0)


class _Scope:
    def __init__(self, on):
        self.on = on
        self.cur = None

    def __call__(self, name):
        if not self.on:
            return
        if self.cur is not None:
            self.cur.__exit__(None, None, None)
        self.cur = None
        if name is not None:
            self.cur = jax.named_scope(name)
            self.cur.__enter__()


DMAS = "x0:1|k0:384|k384:640 x1:2|x2:4 v0:640|x4:8 q0:640"
SCHED = ("w1 l0 bd w2 fk0:3 k0.0:2h w3 fk3:5 l1 k0.2:4 k1.0:3h w4 tx k1.3:4 l2 v0 v1 k2.0:1 w5 fq k2.1:4 v2 l3 k3 "
         "l4 v3 k4 l5 v4 k5 l6 v5 k6 l7 v6 k7 v7 q0 q1 q2 q3 q4 q5 q6 q7")


def make(T=256, FC=512, SC=0, MC=160, LOOP=1, XV=0, GS=3, U=1, XT=1, DEF=1, LAGK=2, LAGV=1, LAGQ=5, RK=6, RN=11, CHK=0,
         EV=4, LNM=0, LG=2, RB=16, DCOL=(512, 128), PT=0, UB=0, LI=2, GR=248, FBK=2, FBQ=2, LAGE=2, CE=0, NW=2, EV0=1, RK0=2, EN=4, PK=0, PN=0, WS=1, DMAS=DMAS, SCHED=SCHED):
    n = S // T
    R = T // 2

    def kernel(x_hbm, wqkv_hbm, wphi_hbm, wo_hbm, w1_hbm, w3_hbm, w2_hbm, out_hbm,
               x_v, wqkv_v, wphi_v, wo_v, w1_v, w3_v, w2_v, a2_v, o_v, wvt_v,
               out_v, sem_i, sem_o, sem_f):
        sc = _Scope(SC)

        def xcp(i0, i1, s):
            return pltpu.make_async_copy(x_hbm.at[pl.ds(i0 * T, (i1 - i0) * T)], x_v.at[pl.ds(i0 * T, (i1 - i0) * T)], sem_i.at[s])

        def wcp(j, c0, c1, s):
            return pltpu.make_async_copy(wqkv_hbm.at[:, pl.ds(j * D + c0, c1 - c0)],
                                         wqkv_v.at[j, :, pl.ds(c0, c1 - c0)], sem_i.at[s])

        def mkcp(tok, s):
            lo, hi = map(int, tok[1:].split(':'))
            return xcp(lo, hi, s) if tok[0] == 'x' else wcp('qkv'.index(tok[0]), lo, hi, s)

        groups = [[pltpu.make_async_copy(wphi_hbm, wphi_v, sem_i.at[0])]]
        for grp in DMAS.split('|'):
            groups.append([mkcp(tok, len(groups)) for tok in grp.split()])
        groups.append([pltpu.make_async_copy(a, b, sem_i.at[len(groups)])
                       for a, b in ((wo_hbm, wo_v), (w1_hbm, w1_v), (w3_hbm, w3_v), (w2_hbm, w2_v))])
        sc('prologue')
        for grp in groups:
            for c in grp:
                c.start()
                pl.semaphore_signal(sem_f, 1)
                pl.semaphore_wait(sem_f, 1)

        def wait(k):
            sc('w%d' % k)
            for c in groups[k]:
                c.wait()
            sc('c%d' % k)

        a2_v[...] = jnp.zeros(a2_v.shape, F32)
        wait(0)
        a2_v[:, 0:DH, :] = wphi_v[...].astype(F32)
        a2 = a2_v[...].reshape(DH * 24, H).astype(BF)
        col = lax.broadcasted_iota(jnp.int32, (H, D), 1)
        hrow = lax.broadcasted_iota(jnp.int32, (H, D), 0)
        xsel = jnp.where((col >= hrow * DH) & (col < hrow * DH + DH), 1.0, 0.0).astype(BF)
        r = _dot(a2, xsel, NN).reshape(DH, 24, D)
        col = lax.broadcasted_iota(jnp.int32, (24, D), 1)
        dcol = col - DH * ((col * 3277) >> 16)
        u = r[0]
        for d in range(1, DH):
            u = jnp.where(dcol == d, r[d], u)
        ub = jnp.concatenate([u, jnp.zeros((8, D), F32)], axis=0).astype(BF)
        bdt = []

        def bd2():
            dup = (lax.broadcasted_iota(jnp.int32, (48, 32), 0) >> 1) == lax.broadcasted_iota(jnp.int32, (48, 32), 1)
            u2 = _dot(jnp.where(dup, 1.0, 0.0).astype(BF), ub, NN)[0:2 * DH].reshape(1, 5, 8, D)
            sh = (NG, 1, 8, D)
            hh = lax.broadcasted_iota(jnp.int32, sh, 0) * 2 + (lax.broadcasted_iota(jnp.int32, sh, 2) & 1)
            cc = lax.broadcasted_iota(jnp.int32, sh, 3)
            msk = (cc >= hh * DH) & (cc < hh * DH + DH)
            bdi = jnp.where(msk, u2, 0.0)
            c16 = lax.broadcasted_iota(jnp.int32, (16, D), 1)
            rows = []
            for g in range(NG):
                if g in SPLIT:
                    rows += [jnp.where((c16 >= 2 * g * DH) & (c16 < 2 * g * DH + DH), u[0:16], 0.0), bdi[g, 4],
                             jnp.where((c16 >= 2 * g * DH + DH) & (c16 < 2 * g * DH + 2 * DH), u[0:16], 0.0)]
                else:
                    rows.append(bdi[g].reshape(2 * DH, D))
            bdf = jnp.concatenate(rows, axis=0)
            for FB, FL in ((FBS[FBQ], FLS[FBQ]), (FBS[FBK], FLS[FBK])):
                bdt.append([bdf[FB[t]:FB[t] + FL[t], 128 * t:128 * (t + 1)].astype(BF) for t in range(5)])

        def fold_part(j, t):
            return _dot(bdt[j][t], wqkv_v[j, :, 128 * t:128 * (t + 1)], NT)

        lnr = [None]

        def ln1(i):
            if LG and i >= LI:
                outs, rs = [], []
                for k in range(T // RB):
                    x = x_v[i * T + k * RB:i * T + (k + 1) * RB, :].astype(F32)
                    c = 1.0 / D if k < LG else jnp.minimum(1.0 / D, rs[k - LG] + 1.0)
                    xc = x - jnp.sum(x, axis=-1, keepdims=True) * c
                    r = lax.rsqrt(jnp.mean(xc * xc, axis=-1, keepdims=True) + 1e-5)
                    rs.append(r)
                    outs.append(xc * r)
                lnr[0] = rs[-1][-8:]
                return jnp.concatenate(outs, axis=0).astype(BF)
            x = x_v[i * T:(i + 1) * T, :].astype(F32)
            xc = x - jnp.mean(x, axis=-1, keepdims=True)
            r = lax.rsqrt(jnp.mean(xc * xc, axis=-1, keepdims=True) + 1e-5)
            lnr[0] = r[GR:GR + 8]
            return (xc * r).astype(BF)

        NP = D // MC
        GP = MC // 40

        phk = [[] for _ in range(n)]
        phq = [[] for _ in range(n)]
        vws = [[] for _ in range(n)]
        kvacc = [None] * NGR
        kvm = [None] * NGR
        W = {}
        xn = {}
        ones8 = jnp.ones((8, T), F32)

        pend = []

        def flush():
            for dst, p, gate in pend:
                for g in range(p.shape[0] // 40):
                    pg = p[40 * g:40 * (g + 1)]
                    dst.append(_phis(pg, NW & 1) if len(dst) in SPLIT else _phi(pg, gate, NW & 1))
            pend.clear()

        def proj(kind, i, c, half=False, gated=False):
            w = W[kind][c]
            if w is None:
                w = wvt_v[c * MC:(c + 1) * MC, :]
            ws = [w[0:MC // 2], w[MC // 2:MC]] if half else [w]
            for w in ws:
                p = _dot(w.astype(BF), xn[i], NT)
                if kind == 'v':
                    vws[i] += [p[40 * g:40 * (g + 1)] for g in range(p.shape[0] // 40)]
                else:
                    gate = jnp.minimum(lnr[0], -3e38).reshape(1, 1, 8, 1) if gated else None
                    pend.append(((phk if kind == 'k' else phq)[i], p, gate))

        rr = lax.broadcasted_iota(jnp.int32, (48, 80), 0)
        pp = lax.broadcasted_iota(jnp.int32, (48, 80), 1)
        hr = jnp.where(((rr >= DH) & (rr < 2 * DH)) | (rr >= 2 * DH + 4), 1, 0)
        mg = hr == (pp & 1)

        lo4 = lax.broadcasted_iota(jnp.int32, (8, T), 0) < 4
        rr = lax.broadcasted_iota(jnp.int32, (64, 128), 0)
        pp = lax.broadcasted_iota(jnp.int32, (64, 128), 1)
        mgs = []
        for s in range(2):
            o0 = 60 if s == 0 else 40
            rh = jnp.where(rr < DH, 0, jnp.where(rr < 2 * DH, 1, 2))
            rh = jnp.where((rr >= o0) & (rr < o0 + 4), rr - o0, rh)
            m0 = 96 if s == 0 else 80
            mix = ((pp >= m0) & (pp < m0 + 8)) | ((pp >= m0 + 24) & (pp < m0 + 32))
            ch = jnp.where(pp < 80, pp & 1, jnp.where(mix & ((pp & 1) != s), 7, 2))
            mgs.append(rh == ch)

        def feat(ph, g):
            a, m, s = GROUPS[g]
            return ph[a] if m is None else jnp.concatenate([ph[a], ph[m][s]], axis=0)

        def kv(i, g):
            a, m, s = GROUPS[g]
            if m is None:
                lhs = [vws[i][a], ones8]
            elif s == 0:
                lhs = [vws[i][a], vws[i][m][0:16], jnp.where(lo4, vws[i][m][16:24], 1.0)]
            else:
                lhs = [vws[i][a], jnp.where(lo4, 1.0, vws[i][m][16:24]), vws[i][m][24:40]]
            new = _dot(jnp.concatenate(lhs, axis=0).astype(BF), feat(phk[i], g), NT)
            kvacc[g] = new if kvacc[g] is None else kvacc[g] + new
            if i == n - 1:
                kvm[g] = jnp.where(mg if m is None else mgs[s], kvacc[g], 0.0).astype(BF)

        nparts = [{} for _ in range(n)]
        tdone = [0] * n

        def nm(i, g):
            a, m, s = GROUPS[g]
            t = _dot(kvm[g], feat(phq[i], g), NN)
            if m is None:
                ra = _rcp(t[40:48] + 1e-6, NW & 2)
                rb = pltpu.roll(ra, 4, 0)
                r0 = jnp.where(lo4, ra, rb)
                r1 = jnp.where(lo4, rb, ra)
                nparts[i][a] = t[0:40] * jnp.concatenate([r0, r0, ra, r1, r1], axis=0)
            else:
                ra = _rcp((t[56:64] if s == 0 else t[40:48]) + 1e-6, NW & 2)
                k0 = 4 if s == 0 else 0
                r0, r1, r2 = [jnp.broadcast_to(ra[k0 + k:k0 + k + 1], (8, T)) for k in range(3)]
                o = t * jnp.concatenate([r0, r0, jnp.where(lo4, r0, r1), r1, r1, r2, r2, r2], axis=0)
                nparts[i][a] = o[0:40]
                if s == 0:
                    nparts[i][m] = o[40:64]
                else:
                    oa = nparts[i][m]
                    nparts[i][m] = jnp.concatenate([oa[0:16], jnp.where(lo4, oa[16:24], o[40:48]), o[48:64]], axis=0)
            if i >= n - PT:
                full = [k for k in range(NG) if k in nparts[i] and nparts[i][k].shape[0] == 40]
                cnt = 0
                while cnt in full:
                    cnt += 1
                for t in range(tdone[i], 40 * cnt // 128):
                    ot = jnp.concatenate([nparts[i][k] for k in range(cnt)], axis=0)[128 * t:128 * (t + 1)]
                    o_v[i * T:(i + 1) * T, 128 * t:128 * (t + 1)] = ot.astype(BF).T
                    tdone[i] = t + 1
            elif g == NGR - 1:
                o_v[i * T:(i + 1) * T, :] = jnp.concatenate([nparts[i][k] for k in range(NG)], axis=0).astype(BF).T

        gdep = [max(a, m or 0) // GP for a, m, s in GROUPS]

        def wsplit(parts, lo, hi, FB, FL):
            m = len(parts)
            w = _overlap_add(parts, FB[:m], FL[:m], FB[m - 1] + FL[m - 1])
            return [w[c * MC:(c + 1) * MC] * LOG2E for c in range(lo, hi)]

        done = {}
        st = {'j': 0, 'kv': 0, 'nm': 0, 'e': 0, 'w': 0}
        kvdone = {}

        def smalls(final=False):
            j = st['j']
            cnt = 0
            ek, rk = (EV0, RK0) if st['w'] < 5 else (EV, RK)
            while st['kv'] < n * NGR and (final or (cnt < rk and j % ek == (ek - 1 + PK) % ek)):
                i, g = divmod(st['kv'], NGR)
                if not final and (done.get(('k', i, gdep[g]), 1 << 20) + LAGK > j or done.get(('v', i, gdep[g]), 1 << 20) + LAGV > j):
                    break
                kv(i, g)
                if i == n - 1:
                    kvdone[g] = j
                st['kv'] += 1
                cnt += 1
            while st['nm'] < n * NGR and (final or (cnt < RN and (st['e'] or j % EN == (EN - 1 + PN) % EN))):
                i, g = divmod(st['nm'], NGR)
                if not final and (kvdone.get(g, 1 << 20) + 1 > j or done.get(('q', i, gdep[g]), 1 << 20) + (LAGE if st['e'] else LAGQ) > j):
                    break
                nm(i, g)
                st['nm'] += 1
                cnt += 1

        parts = {'k': [], 'q': [], 'v': []}
        W['k'], W['q'], W['v'] = [], [], []
        toks = SCHED.split()
        for ti, tok in enumerate(toks):
            nxt = toks[ti + 1] if ti + 1 < len(toks) else ''
            if tok[0] == 'w':
                wait(int(tok[1:]))
                st['w'] = int(tok[1:])
            elif tok[0] == 's':
                sc(tok)
            elif tok[0] == 'f':
                kind = tok[1]
                lo, hi = map(int, tok[2:].split(':')) if len(tok) > 2 else (0, 5)
                parts[kind] += [fold_part('qk'.index(kind), t) for t in range(lo, hi)]
                FB, FL = (FBS[FBQ], FLS[FBQ]) if kind == 'q' else (FBS[FBK], FLS[FBK])
                W[kind] += wsplit(parts[kind], len(W[kind]), FB[hi] // MC if hi < 5 else NP, FB, FL)
                flush()
            elif tok == 'bd':
                bd2()
            elif tok[:2] in ('tv', 'tx'):
                lo, hi = map(int, tok[2:].split(':')) if len(tok) > 2 else (0, 5)
                eye = (lax.broadcasted_iota(jnp.int32, (128, 128), 0) == lax.broadcasted_iota(jnp.int32, (128, 128), 1))
                eye = jnp.where(eye, 1.0, 0.0).astype(BF)
                if tok[1] == 'v':
                    parts['v'] += [_dot(eye, wqkv_v[2, :, t * 128:(t + 1) * 128], NT).astype(BF) for t in range(lo, hi)]
                else:
                    parts['v'] += [wqkv_v[2, :, t * 128:(t + 1) * 128].T for t in range(lo, hi)]
                if WS:
                    for t in range(lo, hi):
                        wvt_v[t * 128:(t + 1) * 128, :] = parts['v'][t]
                    W['v'] += [None for c in range(len(W['v']), 128 * hi // MC)]
                else:
                    wvt = jnp.concatenate(parts['v'], axis=0)
                    W['v'] += [wvt[c * MC:(c + 1) * MC] for c in range(len(W['v']), 128 * hi // MC)]
                flush()
            elif tok[0] == 'l':
                xn[int(tok[1:])] = ln1(int(tok[1:]))
            else:
                nofl = tok.endswith('n')
                gated = tok.endswith('g')
                tok = tok.rstrip('ng')
                half = tok.endswith('h')
                allh = tok.endswith('H')
                t2 = tok.rstrip('hH')
                i = int(t2[1:].split('.')[0])
                lo, hi = map(int, t2.split('.')[1].split(':')) if '.' in t2 else (0, NP)
                for c in range(lo, hi):
                    proj(tok[0], i, c, allh or (half and c == hi - 1), gated)
                    if not (nxt.startswith('w') and c >= hi - DEF) and not nofl:
                        flush()
                    done[(tok[0], i, c)] = st['j']
                    st['e'] = tok[0] == 'q' and i * NP + c >= n * NP - CE
                    smalls()
                    st['j'] += 1
        smalls(True)
        wait(len(groups) - 1)


        def gu(hn, c):
            gate = _dot(hn, w1_v[:, c * FC:(c + 1) * FC], NN)
            up = _dot(hn, w3_v[:, c * FC:(c + 1) * FC], NN)
            hg = 0.5 * gate
            return hg * (jnp.tanh(hg) + 1.0) * up

        def chunk(i):
            rows = [i * T + k * R if isinstance(i, int) else pl.multiple_of(i * T + k * R, R) for k in range(2)]
            orow = [pl.multiple_of(i * R + k * (R // 2), R // 2) for k in range(2)]
            hs, hns = [], []
            for k in range(2):
                h = x_v[pl.ds(rows[k], R), :].astype(F32) + _dot(pltpu.bitcast(o_v[pl.ds(orow[k], R // 2), :], BF) if UB else o_v[pl.ds(rows[k], R), :], wo_v[...], NN)
                hs.append(h)
                hns.append(_ln(h, (lambda: h) if LNM > 1 else None))
            acts = [[], []]
            hb = [hns[k].astype(BF) for k in range(2)]
            for k in range(2):
                for c in range(GS):
                    acts[k].append(gu(hb[k], c).astype(BF))
            if GS < F // FC:
                hf = jnp.concatenate(hns, axis=0).astype(BF)
                for c in range(GS, F // FC):
                    a = gu(hf, c)
                    for k in range(2):
                        acts[k].append(a[k * R:(k + 1) * R].astype(BF))
            for k in range(2):
                c0 = 0
                for cw in (DCOL if k == 1 else (D,)):
                    y = hs[k][:, c0:c0 + cw]
                    for c in range(F // FC):
                        y = y + _dot(acts[k][c], w2_v[c * FC:(c + 1) * FC, c0:c0 + cw], NN)
                    out_v[pl.ds(rows[k], R), c0:c0 + cw] = y.astype(BF)
                    pltpu.make_async_copy(out_v.at[pl.ds(rows[k], R), pl.ds(c0, cw)],
                                          out_hbm.at[pl.ds(rows[k], R), pl.ds(c0, cw)], sem_o).start()
                    c0 += cw

        sc('p2')
        if LOOP:
            def body(j, carry):
                for u in range(U):
                    chunk(j * U + u)
                return carry
            lax.fori_loop(0, n // U, body, 0)
        else:
            for i in range(n):
                chunk(i)
        sc('fin')
        pltpu.make_async_copy(out_v, out_hbm, sem_o).wait()
        sc(None)

    def fn(A_x, A_wqkv, A_w_phi, A_wo, B_x, B_w1, B_w3, B_w2):
        any_spec = pl.BlockSpec(memory_space=pl.ANY)
        out = pl.pallas_call(
            kernel,
            out_shape=jax.ShapeDtypeStruct((S, D), BF),
            in_specs=[any_spec] * 7,
            out_specs=any_spec,
            scratch_shapes=[
                pltpu.VMEM((S, D), BF),
                pltpu.VMEM((3, D, D), BF),
                pltpu.VMEM((DH, DH, H), BF),
                pltpu.VMEM((D, D), BF),
                pltpu.VMEM((D, F), BF),
                pltpu.VMEM((D, F), BF),
                pltpu.VMEM((F, D), BF),
                pltpu.VMEM((DH, 24, H), F32),
                pltpu.VMEM((S // 2, D), jnp.uint32) if UB else pltpu.VMEM((S, D), BF),
                pltpu.VMEM((D, D), BF),
                pltpu.VMEM((S, D), BF),
                pltpu.SemaphoreType.DMA((len(DMAS.split('|')) + 2,)),
                pltpu.SemaphoreType.DMA,
                pltpu.SemaphoreType.REGULAR,
            ],
            compiler_params=pltpu.CompilerParams(vmem_limit_bytes=100 * 1024 * 1024,
                                                 disable_bounds_checks=not CHK, disable_semaphore_checks=not CHK),
        )(A_x.reshape(S, D), A_wqkv, A_w_phi.transpose(1, 2, 0), A_wo, B_w1, B_w3, B_w2)
        return out.reshape(1, S, D)
    return fn


_impl = make()


@jax.jit
def pallas_sequential_preLN__linear_kernel_hedgehog__glu_gated_swiglu__prompt_kernel(
    A_x: jax.Array,
    A_wqkv: jax.Array,
    A_w_phi: jax.Array,
    A_wo: jax.Array,
    B_x: jax.Array,
    B_w1: jax.Array,
    B_w3: jax.Array,
    B_w2: jax.Array,
):
    return _impl(A_x, A_wqkv, A_w_phi, A_wo, B_x, B_w1, B_w3, B_w2)
```

```python
import jax
import jax.numpy as jnp
from jax import lax
import jax.experimental.pallas as pl
import jax.experimental.pallas.tpu as pltpu

S, D, H, DH, F = 2048, 640, 32, 20, 1536
NG = 16
BF = jnp.bfloat16
F32 = jnp.float32
LOG2E = 1.4426950408889634

NT = (((1,), (1,)), ((), ()))
NN = (((1,), (0,)), ((), ()))

FB = (0, 120, 240, 376, 496)
FL = (144, 144, 160, 144, 144)
SPLIT = (1, 3, 6, 9, 12)
GROUPS = ((0, 1, 0), (2, 1, 1), (4, 3, 0), (5, 3, 1), (7, 6, 0), (8, 6, 1), (10, 9, 0), (11, 9, 1),
          (13, 12, 0), (14, 12, 1), (15, None, 0))
NGR = len(GROUPS)


def _dot(a, b, dims):
    return lax.dot_general(a, b, dims, preferred_element_type=F32)


def _ln(x):
    xc = x - jnp.mean(x, axis=-1, keepdims=True)
    return xc * lax.rsqrt(jnp.mean(xc * xc, axis=-1, keepdims=True) + 1e-5)


def _red(x, op, red):
    r = red(x, axis=1)
    r = op(r, pltpu.roll(r, 2, 1))
    r = op(r, pltpu.roll(r, 4, 1))
    return r[:, None]


def _rcp(x):
    r = pl.reciprocal(x, approx=True)
    return r * (2.0 - x * r)


def _phi(p):
    p4 = p.reshape(1, 5, 8, p.shape[1])
    mx = _red(p4, jnp.maximum, jnp.max)
    mn = _red(p4, jnp.minimum, jnp.min)
    ep = jnp.exp2(p4 - mx)
    en = jnp.exp2(mn - p4)
    sp = _red(ep, jnp.add, jnp.sum)
    sn = _red(en, jnp.add, jnp.sum)
    r = _rcp(sp * sn)
    return jnp.concatenate([ep * (r * sn), en * (r * sp)], axis=1).reshape(80, p.shape[1]).astype(BF)


def _phis(p):
    ev = (lax.broadcasted_iota(jnp.int32, (8, p.shape[1]), 0) & 1) == 0

    def red(v, op):
        a, b = op(v[0], v[1]), op(v[3], v[4])
        c = op(jnp.where(ev, a, b), pltpu.roll(jnp.where(ev, b, a), 1, 0))
        c = op(c, v[2])
        c = op(c, pltpu.roll(c, 2, 0))
        return op(c, pltpu.roll(c, 4, 0))

    def spread(c):
        cr = pltpu.roll(c, 1, 0)
        a, b = jnp.where(ev, c, cr), jnp.where(ev, cr, c)
        return [a, a, c, b, b]

    v = [p[8 * j:8 * (j + 1)] for j in range(5)]
    mx, mn = red(v, jnp.maximum), red(v, jnp.minimum)
    ep = [jnp.exp2(x - m) for x, m in zip(v, spread(mx))]
    en = [jnp.exp2(m - x) for x, m in zip(v, spread(mn))]
    sp, sn = red(ep, jnp.add), red(en, jnp.add)
    r = _rcp(sp * sn)
    ep = [x * m for x, m in zip(ep, spread(r * sn))]
    en = [x * m for x, m in zip(en, spread(r * sp))]
    return [jnp.concatenate(ep[0:3] + en[0:3], axis=0).astype(BF), jnp.concatenate(ep[2:5] + en[2:5], axis=0).astype(BF)]


def _overlap_add(parts, bases, lens, total):
    cuts = sorted(set([0, total] + list(bases) + [b + l for b, l in zip(bases, lens)]))
    out = []
    for lo, hi in zip(cuts[:-1], cuts[1:]):
        acc = None
        for p, b, l in zip(parts, bases, lens):
            if b <= lo and hi <= b + l:
                piece = p[lo - b:hi - b]
                acc = piece if acc is None else acc + piece
        out.append(acc)
    return jnp.concatenate(out, axis=0)


class _Scope:
    def __init__(self, on):
        self.on = on
        self.cur = None

    def __call__(self, name):
        if not self.on:
            return
        if self.cur is not None:
            self.cur.__exit__(None, None, None)
        self.cur = None
        if name is not None:
            self.cur = jax.named_scope(name)
            self.cur.__enter__()


DMAS = "x0:1|k0:384|k384:640 x1:2|v0:640 x2:3|x3:8 q0:640"
SCHED = ("w1 l0 bd w2 fk0:3 k0.0:2h w3 fk3:5 l1 k0.2:4 k1.0:3h w4 tx k1.3:4 l2 v0 v1 k2.0:1 w5 k2.1:4 fq v2 l3 k3 "
         "l4 v3 k4 l5 v4 k5 l6 v5 k6 l7 v6 k7 v7 q0 q1 q2 q3 q4 q5 q6 q7")


def make(T=256, FC=512, SC=0, MC=160, DEF=1, LAGK=2, LAGV=1, LAGQ=5, RK=4, RN=22, CHK=0, EV=4, LG=2, RB=16,
         DCOL=(512, 128), LI=2, EV0=1, RK0=2, EN=8, DMAS=DMAS, SCHED=SCHED):
    n = S // T
    R = T // 2

    def kernel(x_hbm, wqkv_hbm, wphi_hbm, wo_hbm, w1_hbm, w3_hbm, w2_hbm, out_hbm,
               x_v, wqkv_v, wphi_v, wo_v, w1_v, w3_v, w2_v, a2_v, o_v, wvt_v, ot_v,
               out_v, sem_i, sem_o, sem_f):
        sc = _Scope(SC)

        def xcp(i0, i1, s):
            return pltpu.make_async_copy(x_hbm.at[pl.ds(i0 * T, (i1 - i0) * T)], x_v.at[pl.ds(i0 * T, (i1 - i0) * T)], sem_i.at[s])

        def wcp(j, c0, c1, s):
            return pltpu.make_async_copy(wqkv_hbm.at[:, pl.ds(j * D + c0, c1 - c0)],
                                         wqkv_v.at[j, :, pl.ds(c0, c1 - c0)], sem_i.at[s])

        def mkcp(tok, s):
            lo, hi = map(int, tok[1:].split(':'))
            return xcp(lo, hi, s) if tok[0] == 'x' else wcp('qkv'.index(tok[0]), lo, hi, s)

        groups = [[pltpu.make_async_copy(wphi_hbm, wphi_v, sem_i.at[0])]]
        for grp in DMAS.split('|'):
            groups.append([mkcp(tok, len(groups)) for tok in grp.split()])
        groups.append([pltpu.make_async_copy(a, b, sem_i.at[len(groups)])
                       for a, b in ((wo_hbm, wo_v), (w1_hbm, w1_v), (w3_hbm, w3_v), (w2_hbm, w2_v))])
        sc('prologue')
        for grp in groups:
            for c in grp:
                c.start()
                pl.semaphore_signal(sem_f, 1)
                pl.semaphore_wait(sem_f, 1)

        def wait(k):
            sc('w%d' % k)
            for c in groups[k]:
                c.wait()
            sc('c%d' % k)

        a2_v[...] = jnp.zeros(a2_v.shape, F32)
        o_v[(n - 1) * T:n * T, :] = jnp.zeros((T, D), BF)
        wait(0)
        a2_v[:, 0:DH, :] = wphi_v[...].astype(F32)
        a2 = a2_v[...].reshape(DH * 24, H).astype(BF)
        col = lax.broadcasted_iota(jnp.int32, (H, D), 1)
        hrow = lax.broadcasted_iota(jnp.int32, (H, D), 0)
        xsel = jnp.where((col >= hrow * DH) & (col < hrow * DH + DH), 1.0, 0.0).astype(BF)
        r = _dot(a2, xsel, NN).reshape(DH, 24, D)
        col = lax.broadcasted_iota(jnp.int32, (24, D), 1)
        dcol = col - DH * ((col * 3277) >> 16)
        u = r[0]
        for d in range(1, DH):
            u = jnp.where(dcol == d, r[d], u)
        ub = jnp.concatenate([u, jnp.zeros((8, D), F32)], axis=0).astype(BF)
        bdt = []

        def bd2():
            dup = (lax.broadcasted_iota(jnp.int32, (48, 32), 0) >> 1) == lax.broadcasted_iota(jnp.int32, (48, 32), 1)
            u2 = _dot(jnp.where(dup, 1.0, 0.0).astype(BF), ub, NN)[0:2 * DH].reshape(1, 5, 8, D)
            sh = (NG, 1, 8, D)
            hh = lax.broadcasted_iota(jnp.int32, sh, 0) * 2 + (lax.broadcasted_iota(jnp.int32, sh, 2) & 1)
            cc = lax.broadcasted_iota(jnp.int32, sh, 3)
            msk = (cc >= hh * DH) & (cc < hh * DH + DH)
            bdi = jnp.where(msk, u2, 0.0)
            c16 = lax.broadcasted_iota(jnp.int32, (16, D), 1)
            rows = []
            for g in range(NG):
                if g in SPLIT:
                    rows += [jnp.where((c16 >= 2 * g * DH) & (c16 < 2 * g * DH + DH), u[0:16], 0.0), bdi[g, 4],
                             jnp.where((c16 >= 2 * g * DH + DH) & (c16 < 2 * g * DH + 2 * DH), u[0:16], 0.0)]
                else:
                    rows.append(bdi[g].reshape(2 * DH, D))
            bdf = jnp.concatenate(rows, axis=0)
            bdt.extend(bdf[FB[t]:FB[t] + FL[t], 128 * t:128 * (t + 1)].astype(BF) for t in range(5))

        def fold_part(j, t):
            return _dot(bdt[t], wqkv_v[j, :, 128 * t:128 * (t + 1)], NT)

        def ln1(i):
            if LG and i >= LI:
                outs, rs = [], []
                for k in range(T // RB):
                    x = x_v[i * T + k * RB:i * T + (k + 1) * RB, :].astype(F32)
                    c = 1.0 / D if k < LG else jnp.minimum(1.0 / D, rs[k - LG] + 1.0)
                    xc = x - jnp.sum(x, axis=-1, keepdims=True) * c
                    r = lax.rsqrt(jnp.mean(xc * xc, axis=-1, keepdims=True) + 1e-5)
                    rs.append(r)
                    outs.append(xc * r)
                return jnp.concatenate(outs, axis=0).astype(BF)
            x = x_v[i * T:(i + 1) * T, :].astype(F32)
            xc = x - jnp.mean(x, axis=-1, keepdims=True)
            r = lax.rsqrt(jnp.mean(xc * xc, axis=-1, keepdims=True) + 1e-5)
            return (xc * r).astype(BF)

        NP = D // MC
        GP = MC // 40

        phk = [{} for _ in range(n)]
        phq = [{} for _ in range(n)]
        vws = [[] for _ in range(n)]
        kvacc = [None] * NGR
        kvm = [None] * NGR
        W = {}
        xn = {}
        ones8 = jnp.ones((8, T), F32)

        pend = []

        def flush():
            for dst, base, p in pend:
                for g in range(p.shape[0] // 40):
                    dst[base + g] = (_phis if base + g in SPLIT else _phi)(p[40 * g:40 * (g + 1)])
            pend.clear()

        def proj(kind, i, c, half):
            w = wvt_v[c * MC:(c + 1) * MC, :] if kind == 'v' else W[kind][c]
            for hi, w in enumerate([w[0:MC // 2], w[MC // 2:MC]] if half else [w]):
                p = _dot(w.astype(BF), xn[i], NT)
                if kind == 'v':
                    vws[i] += [p[40 * g:40 * (g + 1)] for g in range(p.shape[0] // 40)]
                else:
                    pend.append(((phk if kind == 'k' else phq)[i], c * GP + hi * GP // 2, p))

        rr = lax.broadcasted_iota(jnp.int32, (48, 80), 0)
        pp = lax.broadcasted_iota(jnp.int32, (48, 80), 1)
        hr = jnp.where(((rr >= DH) & (rr < 2 * DH)) | (rr >= 2 * DH + 4), 1, 0)
        mg = hr == (pp & 1)

        lo4 = lax.broadcasted_iota(jnp.int32, (8, T), 0) < 4
        rr = lax.broadcasted_iota(jnp.int32, (64, 128), 0)
        pp = lax.broadcasted_iota(jnp.int32, (64, 128), 1)
        mgs = []
        for s in range(2):
            o0 = 60 if s == 0 else 40
            rh = jnp.where(rr < DH, 0, jnp.where(rr < 2 * DH, 1, 2))
            rh = jnp.where((rr >= o0) & (rr < o0 + 4), rr - o0, rh)
            m0 = 96 if s == 0 else 80
            mix = ((pp >= m0) & (pp < m0 + 8)) | ((pp >= m0 + 24) & (pp < m0 + 32))
            ch = jnp.where(pp < 80, pp & 1, jnp.where(mix & ((pp & 1) != s), 7, 2))
            mgs.append(rh == ch)

        def feat(ph, g):
            a, m, s = GROUPS[g]
            return ph[a] if m is None else jnp.concatenate([ph[a], ph[m][s]], axis=0)

        def kv(i, g):
            a, m, s = GROUPS[g]
            if m is None:
                lhs = [vws[i][a], ones8]
            elif s == 0:
                lhs = [vws[i][a], vws[i][m][0:16], jnp.where(lo4, vws[i][m][16:24], 1.0)]
            else:
                lhs = [vws[i][a], jnp.where(lo4, 1.0, vws[i][m][16:24]), vws[i][m][24:40]]
            new = _dot(jnp.concatenate(lhs, axis=0).astype(BF), feat(phk[i], g), NT)
            kvacc[g] = new if kvacc[g] is None else kvacc[g] + new
            if i == n - 1:
                kvm[g] = jnp.where(mg if m is None else mgs[s], kvacc[g], 0.0).astype(BF)

        nparts = [{} for _ in range(n)]
        sdone = set()

        def nm(i, g):
            a, m, s = GROUPS[g]
            t = _dot(kvm[g], feat(phq[i], g), NN)
            if m is None:
                ra = _rcp(t[40:48] + 1e-6)
                rb = pltpu.roll(ra, 4, 0)
                r0 = jnp.where(lo4, ra, rb)
                r1 = jnp.where(lo4, rb, ra)
                nparts[i][a] = t[0:40] * jnp.concatenate([r0, r0, ra, r1, r1], axis=0)
            else:
                ra = _rcp((t[56:64] if s == 0 else t[40:48]) + 1e-6)
                k0 = 4 if s == 0 else 0
                r0, r1, r2 = [jnp.broadcast_to(ra[k0 + k:k0 + k + 1], (8, T)) for k in range(3)]
                o = t * jnp.concatenate([r0, r0, jnp.where(lo4, r0, r1), r1, r1, r2, r2, r2], axis=0)
                nparts[i][a] = o[0:40]
                if s == 0:
                    nparts[i][m] = o[40:64]
                else:
                    oa = nparts[i][m]
                    nparts[i][m] = jnp.concatenate([oa[0:16], jnp.where(lo4, oa[16:24], o[40:48]), o[48:64]], axis=0)
            if i == n - 1:
                full = [k for k in range(NG) if k in nparts[i] and nparts[i][k].shape[0] == 40]
                for k2 in range(NG // 2):
                    if 2 * k2 in full and 2 * k2 + 1 in full and k2 not in sdone:
                        sdone.add(k2)
                        ot_v[80 * k2:80 * (k2 + 1), :] = jnp.concatenate(
                            [nparts[i][2 * k2], nparts[i][2 * k2 + 1]], axis=0).astype(BF)
            elif g == NGR - 1:
                o_v[i * T:(i + 1) * T, :] = jnp.concatenate([nparts[i][k] for k in range(NG)], axis=0).astype(BF).T

        gdep = [max(a, m or 0) // GP for a, m, s in GROUPS]

        def wsplit(parts, lo, hi):
            m = len(parts)
            w = _overlap_add(parts, FB[:m], FL[:m], FB[m - 1] + FL[m - 1])
            return [w[c * MC:(c + 1) * MC] * LOG2E for c in range(lo, hi)]

        done = {}
        st = {'j': 0, 'kv': 0, 'nm': 0, 'w': 0}
        kvdone = {}

        def smalls(final=False):
            j = st['j']
            cnt = 0
            ek, rk = (EV0, RK0) if st['w'] < 5 else (EV, RK)
            while st['kv'] < n * NGR and (final or (cnt < rk and j % ek == ek - 1)):
                i, g = divmod(st['kv'], NGR)
                if not final and (done.get(('k', i, gdep[g]), 1 << 20) + LAGK > j or done.get(('v', i, gdep[g]), 1 << 20) + LAGV > j):
                    break
                kv(i, g)
                if i == n - 1:
                    kvdone[g] = j
                st['kv'] += 1
                cnt += 1
            while st['nm'] < n * NGR and (final or (cnt < RN and j % EN == EN - 1)):
                i, g = divmod(st['nm'], NGR)
                if not final and (kvdone.get(g, 1 << 20) + 1 > j or done.get(('q', i, gdep[g]), 1 << 20) + LAGQ > j):
                    break
                nm(i, g)
                st['nm'] += 1
                cnt += 1

        parts = {'k': [], 'q': []}
        W['k'], W['q'] = [], []
        toks = SCHED.split()
        for ti, tok in enumerate(toks):
            nxt = toks[ti + 1] if ti + 1 < len(toks) else ''
            if tok[0] == 'w':
                wait(int(tok[1:]))
                st['w'] = int(tok[1:])
            elif tok[0] == 'f':
                kind = tok[1]
                lo, hi = map(int, tok[2:].split(':')) if len(tok) > 2 else (0, 5)
                parts[kind] += [fold_part('qk'.index(kind), t) for t in range(lo, hi)]
                W[kind] += wsplit(parts[kind], len(W[kind]), FB[hi] // MC if hi < 5 else NP)
                flush()
            elif tok == 'bd':
                bd2()
            elif tok == 'tx':
                for t in range(5):
                    wvt_v[t * 128:(t + 1) * 128, :] = wqkv_v[2, :, t * 128:(t + 1) * 128].T
                flush()
            elif tok[0] == 'l':
                xn[int(tok[1:])] = ln1(int(tok[1:]))
            else:
                half = tok.endswith('h')
                t2 = tok.rstrip('h')
                i = int(t2[1:].split('.')[0])
                lo, hi = map(int, t2.split('.')[1].split(':')) if '.' in t2 else (0, NP)
                for c in range(lo, hi):
                    proj(tok[0], i, c, half and c == hi - 1)
                    if not (nxt.startswith('w') and c >= hi - DEF):
                        flush()
                    done[(tok[0], i, c)] = st['j']
                    smalls()
                    st['j'] += 1
        smalls(True)
        wait(len(groups) - 1)


        def gu(hn, c):
            gate = _dot(hn, w1_v[:, c * FC:(c + 1) * FC], NN)
            up = _dot(hn, w3_v[:, c * FC:(c + 1) * FC], NN)
            hg = 0.5 * gate
            return hg * (jnp.tanh(hg) + 1.0) * up

        def chunk(i, carry):
            rows = [pl.multiple_of(i * T + k * R, R) for k in range(2)]
            hs = [x_v[pl.ds(rows[k], R), :].astype(F32) + _dot(o_v[pl.ds(rows[k], R), :], wo_v[...], NN)
                  for k in range(2)]
            o_v[(n - 1) * T:n * T, :] = ot_v[...].T
            acts = [[gu(_ln(hs[k]).astype(BF), c).astype(BF) for c in range(F // FC)] for k in range(2)]
            for k in range(2):
                c0 = 0
                for cw in (DCOL if k == 1 else (D,)):
                    y = hs[k][:, c0:c0 + cw]
                    for c in range(F // FC):
                        y = y + _dot(acts[k][c], w2_v[c * FC:(c + 1) * FC, c0:c0 + cw], NN)
                    out_v[pl.ds(rows[k], R), c0:c0 + cw] = y.astype(BF)
                    pltpu.make_async_copy(out_v.at[pl.ds(rows[k], R), pl.ds(c0, cw)],
                                          out_hbm.at[pl.ds(rows[k], R), pl.ds(c0, cw)], sem_o).start()
                    c0 += cw
            return carry

        sc('p2')
        lax.fori_loop(0, n, chunk, 0)
        sc('fin')
        pltpu.make_async_copy(out_v, out_hbm, sem_o).wait()
        sc(None)

    def fn(A_x, A_wqkv, A_w_phi, A_wo, B_x, B_w1, B_w3, B_w2):
        any_spec = pl.BlockSpec(memory_space=pl.ANY)
        out = pl.pallas_call(
            kernel,
            out_shape=jax.ShapeDtypeStruct((S, D), BF),
            in_specs=[any_spec] * 7,
            out_specs=any_spec,
            scratch_shapes=[
                pltpu.VMEM((S, D), BF),
                pltpu.VMEM((3, D, D), BF),
                pltpu.VMEM((DH, DH, H), BF),
                pltpu.VMEM((D, D), BF),
                pltpu.VMEM((D, F), BF),
                pltpu.VMEM((D, F), BF),
                pltpu.VMEM((F, D), BF),
                pltpu.VMEM((DH, 24, H), F32),
                pltpu.VMEM((S, D), BF),
                pltpu.VMEM((D, D), BF),
                pltpu.VMEM((D, T), BF),
                pltpu.VMEM((S, D), BF),
                pltpu.SemaphoreType.DMA((len(DMAS.split('|')) + 2,)),
                pltpu.SemaphoreType.DMA,
                pltpu.SemaphoreType.REGULAR,
            ],
            compiler_params=pltpu.CompilerParams(vmem_limit_bytes=100 * 1024 * 1024,
                                                 disable_bounds_checks=not CHK, disable_semaphore_checks=not CHK),
        )(A_x.reshape(S, D), A_wqkv, A_w_phi.transpose(1, 2, 0), A_wo, B_w1, B_w3, B_w2)
        return out.reshape(1, S, D)
    return fn


_impl = make()


@jax.jit
def pallas_sequential_preLN__linear_kernel_hedgehog__glu_gated_swiglu__prompt_kernel(
    A_x: jax.Array,
    A_wqkv: jax.Array,
    A_w_phi: jax.Array,
    A_wo: jax.Array,
    B_x: jax.Array,
    B_w1: jax.Array,
    B_w3: jax.Array,
    B_w2: jax.Array,
):
    return _impl(A_x, A_wqkv, A_w_phi, A_wo, B_x, B_w1, B_w3, B_w2)
```
